```python
import jax
import jax.numpy as jnp

def _softmax(x, axis=-1):
    return jax.nn.softmax(x, axis=axis)
def _gelu(x):
    return jax.nn.gelu(x, approximate=True)
def _silu(x):
    return jax.nn.silu(x)
def _sigmoid(x):
    return jax.nn.sigmoid(x)
def _layernorm(x, axis=-1, eps=1e-5):
    m = jnp.mean(x, axis=axis, keepdims=True)
    v = jnp.var(x, axis=axis, keepdims=True)
    return (x - m) / jnp.sqrt(v + eps)
def _scatter_add(tgt, idx, src, axis=0):
    return tgt.at[idx].add(src)
def _segment_sum(src, seg, n):
    return jax.ops.segment_sum(src, seg, n)
class _Rng:
    def __init__(self, key):
        self._k = key
    def _next(self):
        self._k, sub = jax.random.split(self._k)
        return sub
    def normal(self, shape):
        return jax.random.normal(self._next(), shape, dtype=jnp.bfloat16)
    def randint(self, lo, hi, shape):
        return jax.random.randint(self._next(), shape, lo, hi, dtype=jnp.int32)
    def uniform(self, shape, lo=0.0, hi=1.0):
        return jax.random.uniform(self._next(), shape, jnp.bfloat16, lo, hi)
    def permutation(self, n):
        return jax.random.permutation(self._next(), n)


kernel_name = 'gated_mix__compressed_kv_cla__ssm_conv_h3__prompt'

def setup_inputs():
    _rng = _Rng(jax.random.key(int.from_bytes(__import__("os").urandom(4), "little")))
    _w = (lambda a: (lambda t: t.astype(jnp.bfloat16) if jnp.issubdtype(t.dtype, jnp.floating) else t)(jnp.asarray(a)))
    def _A_setup():
        B, H, Sq, Sk, D, M = 1, 32, 2048, 2048, 128, 1024
        Dc = 4 * D
        return {
            "x": _w((lambda *s: _rng.normal(s) * 0.05)(B, Sq, M)),
            "c_kv": _w((lambda *s: _rng.normal(s) * 0.05)(B, Sk, Dc)),
            "w_q": _w((lambda *s: _rng.normal(s) * 0.05)(M, H, D) * (M ** -0.5)),
            "w_uk": _w((lambda *s: _rng.normal(s) * 0.05)(Dc, H, D) * (Dc ** -0.5)),
            "w_uv": _w((lambda *s: _rng.normal(s) * 0.05)(Dc, H, D) * (Dc ** -0.5)),
            "w_o": _w((lambda *s: _rng.normal(s) * 0.05)(H, D, M) * ((H * D) ** -0.5)),
        }
    _A_in = _A_setup()

    def _B_setup():
        B, S, D = 1, 2048, 1024
        ks = 4
        return {
            "q": _w((lambda *s: _rng.normal(s) * 0.05)(B, S, D)),
            "k": _w((lambda *s: _rng.normal(s) * 0.05)(B, S, D)),
            "v": _w((lambda *s: _rng.normal(s) * 0.05)(B, S, D)),
            "shift_k": _w((lambda *s: _rng.normal(s) * 0.05)(D, ks) * 0.5),
            "ssm_k": _w((lambda *s: _rng.normal(s) * 0.05)(D, S) * (1.0 / S ** 0.5)),
            "ssm_D": _w((lambda *s: _rng.normal(s) * 0.05)(D)),
        }
    _B_in = _B_setup()

    return {
        "A_x": _A_in["x"],
        "A_c_kv": _A_in["c_kv"],
        "A_w_q": _A_in["w_q"],
        "A_w_uk": _A_in["w_uk"],
        "A_w_uv": _A_in["w_uv"],
        "A_w_o": _A_in["w_o"],
        "B_q": _B_in["q"],
        "B_k": _B_in["k"],
        "B_v": _B_in["v"],
        "B_shift_k": _B_in["shift_k"],
        "B_ssm_k": _B_in["ssm_k"],
        "B_ssm_D": _B_in["ssm_D"],
        "gate_w": _w((lambda *s: _rng.normal(s) * 0.05)(1024)),
    }

def reference(A_x, A_c_kv, A_w_q, A_w_uk, A_w_uv, A_w_o, B_q, B_k, B_v, B_shift_k, B_ssm_k, B_ssm_D, gate_w):
    def _A_ref(x, c_kv, w_q, w_uk, w_uv, w_o):
        B, Sq, M = x.shape[0], x.shape[1], x.shape[2]
        Sk = c_kv.shape[1]
        H, D = w_q.shape[1], w_q.shape[2]
        q = jnp.einsum("bqm,mhd->bhqd", x, w_q)
        k = jnp.einsum("bkc,chd->bhkd", c_kv, w_uk)
        v = jnp.einsum("bkc,chd->bhkd", c_kv, w_uv)
        scores = jnp.einsum("bhqd,bhkd->bhqk", q, k) * (D ** -0.5)
        off = Sk - Sq
        qi = jnp.arange(Sq)[:, None]
        kj = jnp.arange(Sk)[None, :]
        cmask = kj <= (qi + off)
        scores = jnp.where(cmask[None, None], scores, -1e9)
        p = _softmax(scores, axis=-1)
        ctx = jnp.einsum("bhqk,bhkd->bhqd", p, v)
        return jnp.einsum("bhqd,hdm->bqm", ctx, w_o)

    def _B_ref(q, k, v, shift_k, ssm_k, ssm_D):
        B, S, D = q.shape
        ks = shift_k.shape[-1]
        k_pad = jnp.pad(k, ((0, 0), (ks - 1, 0), (0, 0)))
        k_shift = jnp.zeros_like(k)
        for t in range(ks):
            k_shift = k_shift + k_pad[:, t:t + S, :] * shift_k[:, ks - 1 - t][None, None, :]
        kv = k_shift * v
        L = 2 * S
        kv_pad = jnp.pad(kv, ((0, 0), (0, S), (0, 0)))
        kf_pad = jnp.pad(ssm_k, ((0, 0), (0, S)))
        kv_f = (lambda x, axes=(-2,-1): jnp.fft.rfft2(x.astype(jnp.float32), axes=axes))(kv_pad[:, None, :, :], axes=(1, 2))
        kf_f = (lambda x, axes=(-2,-1): jnp.fft.rfft2(x.astype(jnp.float32), axes=axes))(kf_pad[:, None, :], axes=(1, 2))
        kf_f = (lambda x, *d: x.transpose(*d))(kf_f, 1, 2, 0)
        y_f = kv_f * kf_f[None, :, :, :]
        y = (lambda x, s, axes=(-2,-1): jnp.fft.irfft2(x, s=s, axes=axes).astype(jnp.bfloat16))(y_f, (1, L), axes=(1, 2))[:, 0, :S, :]
        y = y + kv * ssm_D[None, None, :]
        return q * y

    x = A_x
    g = _sigmoid((x * gate_w).sum(-1, keepdims=True))
    a = _A_ref(x, A_c_kv, A_w_q, A_w_uk, A_w_uv, A_w_o)
    b = _B_ref(x, B_k, B_v, B_shift_k, B_ssm_k, B_ssm_D)
    return g * a + (1 - g) * b
```

```python
import numpy as np
import jax
import jax.numpy as jnp
from jax import lax
import jax.experimental.pallas as pl
import jax.experimental.pallas.tpu as pltpu

S, M, H, D, C = 2048, 1024, 32, 128, 512
G = 8
P = G // 2
T = 128
TQ = 256
NB = S // TQ
NC = S // T
KS = 4
NEG = -1e9
QSCALE = float(D ** -0.5 * np.log2(np.e))
bf16 = jnp.bfloat16
f32 = jnp.float32
u32 = jnp.uint32


def _nt(a, b):
    return lax.dot_general(a, b, (((1,), (1,)), ((), ())), preferred_element_type=f32)


def _nn(a, b):
    return jnp.dot(a, b, preferred_element_type=f32)


def _unpack_pair(w32):
    lo = lax.bitcast_convert_type(w32 << 16, f32).astype(bf16)
    hi = lax.bitcast_convert_type(w32 & u32(0xFFFF0000), f32).astype(bf16)
    return jnp.concatenate([lo, hi], axis=1)


def _convert_group(w_ref, w32, rows):
    ch = 64

    def body(c, _):
        r = pl.multiple_of(c * ch, ch)
        v = w_ref[pl.ds(r, ch), :, :]
        w32[pl.ds(pl.multiple_of(c * ch * P, ch * P), ch * P), :] = pltpu.bitcast(
            v.reshape(ch * G, D), u32)
        return 0

    lax.fori_loop(0, rows // ch, body, 0)


def _recip(l):
    r = pl.reciprocal(l, approx=True)
    return r * (2.0 - l * r)


def _dft_tables():
    n = np.arange(T)[None, :]
    k = np.arange(T)[:, None]
    ang = 2.0 * np.pi * ((n * (2 * k + 1)) % (4 * T)) / (4 * T)
    cos, sin = np.cos(ang), np.sin(ang)
    hf = T // 2
    fwd = np.stack([np.concatenate([cos[h * hf:(h + 1) * hf], -sin[h * hf:(h + 1) * hf]], axis=0)
                    for h in range(2)])
    inv = np.transpose(fwd, (0, 2, 1)) / T
    return fwd.astype(np.float32), inv.astype(np.float32)


def _kernel(x_ref, c_ref, wq_ref, wuk_ref, wuv_ref, wo_ref,
            xt_ref, bk_ref, bv_ref, sh_ref, sk_ref, sd_ref, gw_ref, f_ref, gi_ref,
            o_ref,
            wq32, wuk32, wuv32, acc, kpad, ybuf, bbuf, gbuf):
    s = pl.program_id(0)

    @pl.when(s % P == 0)
    def _():
        _convert_group(wq_ref, wq32, M)
        _convert_group(wuk_ref, wuk32, C)
        _convert_group(wuv_ref, wuv32, C)

    @pl.when(s == 0)
    def _():
        acc[...] = jnp.zeros_like(acc)
        kpad[0:8, :] = jnp.zeros((8, T), f32)

    i0 = s % P
    wq = _unpack_pair(wq32[pl.ds(i0, M, stride=P), :])
    wuk = _unpack_pair(wuk32[pl.ds(i0, C, stride=P), :])
    wuv = _unpack_pair(wuv32[pl.ds(i0, C, stride=P), :])
    wo = wo_ref[...].reshape(2 * D, M)
    row = lax.broadcasted_iota(jnp.int32, (T, T), 0)
    col = lax.broadcasted_iota(jnp.int32, (T, T), 1)
    mask = col <= row

    def qproj(i):
        return (_nn(x_ref[i * TQ:(i + 1) * TQ, :], wq) * QSCALE).astype(bf16)

    def scores(q, k):
        w = k.shape[0]
        s1 = _nt(q, k[0:w - T])
        s2 = _nt(q[T:], k[w - T:w])
        top_d = jnp.where(mask, s1[:T, w - 2 * T:], NEG)
        top = jnp.concatenate([s1[:T, :w - 2 * T], top_d], axis=1) if w > 2 * T else top_d
        bot = jnp.concatenate([s1[T:, :], jnp.where(mask, s2, NEG)], axis=1)
        return top, bot

    def softmax(sc):
        m = jnp.max(sc, axis=1, keepdims=True)
        p = jnp.exp2(sc - m)
        l = jnp.sum(p, axis=1, keepdims=True)
        return p.astype(bf16), l

    def pv(sc, v):
        top, bot = sc
        w = v.shape[0]
        pt, lt = softmax(top)
        pb, lb = softmax(bot)
        p1 = jnp.concatenate([pt, pb[:, :w - T]], axis=0)
        o1 = _nn(p1, v[0:w - T])
        o2 = _nn(pb[:, w - T:], v[w - T:w])
        ot = o1[:T] * _recip(lt)
        ob = (o1[T:] + o2) * _recip(lb)
        return jnp.concatenate([ot, ob], axis=0).astype(bf16)

    def oproj(i, ctx2):
        acc[i * TQ:(i + 1) * TQ, :] += _nn(ctx2, wo)

    hf = T // 2
    st = {}

    def b_input():
        eye = (lax.broadcasted_iota(jnp.int32, (16, KS), 0)
               == lax.broadcasted_iota(jnp.int32, (16, KS), 1)).astype(bf16)
        taps = _nt(eye, sh_ref[...])
        kf = bk_ref[...].astype(f32)
        kpad[8:8 + S, :] = kf
        ks = kf * taps[0:1, :]
        for j in range(1, KS):
            ks = ks + kpad[8 - j:8 - j + S, :] * taps[j:j + 1, :]
        u = ks * bv_ref[...].astype(f32)
        st["u"] = u
        ub = u.astype(bf16)
        st["ub"] = jnp.concatenate([ub[a * T:(a + 1) * T, :] for a in range(NC)], axis=1)

    def b_forward():
        fm = f_ref[...]
        uh = _nn(fm, st["ub"])
        hs = jnp.concatenate([sk_ref[:, j * T:(j + 1) * T] for j in range(NC)], axis=0)
        hh = _nt(fm, hs)
        sgn = jnp.where(lax.broadcasted_iota(jnp.int32, (hf, T), 0) % 2 == 0, 1.0, -1.0)
        ur = [uh[0:hf, a * T:(a + 1) * T] for a in range(NC)]
        ui = [uh[hf:T, a * T:(a + 1) * T] for a in range(NC)]
        hr0 = [hh[0:hf, a * T:(a + 1) * T] for a in range(NC)]
        hi0 = [hh[hf:T, a * T:(a + 1) * T] for a in range(NC)]
        hr = [hr0[0]] + [hr0[j] - sgn * hi0[j - 1] for j in range(1, NC)]
        hi = [hi0[0]] + [hi0[j] + sgn * hr0[j - 1] for j in range(1, NC)]
        st["ur"], st["ui"] = ur, ui
        st["us"] = [ur[a] + ui[a] for a in range(NC)]
        st["hr"] = hr
        st["hd"] = [hi[j] - hr[j] for j in range(NC)]
        st["hs"] = [hr[j] + hi[j] for j in range(NC)]

    def b_mac(c):
        k1 = k2 = k3 = None
        for a in range(c + 1):
            j = c - a
            t1 = st["hr"][j] * st["us"][a]
            t2 = st["ur"][a] * st["hd"][j]
            t3 = st["ui"][a] * st["hs"][j]
            k1 = t1 if k1 is None else k1 + t1
            k2 = t2 if k2 is None else k2 + t2
            k3 = t3 if k3 is None else k3 + t3
        z = jnp.concatenate([k1 - k3, k1 + k2], axis=0).astype(bf16)
        rows = slice(c * T, (c + 1) * T)
        y = _nn(gi_ref[...], z)
        y = y + jnp.where(s % 2 == 1, ybuf[rows, :], 0.0)
        ybuf[rows, :] = y
        bbuf[s // 2, rows, :] = xt_ref[rows, :].astype(f32) * (
            y + st["u"][rows, :] * sd_ref[...].astype(f32))

    def gate():
        r = pl.multiple_of(s * T, T)
        xg = x_ref[pl.ds(r, T), :].astype(f32) * gw_ref[...].astype(f32)
        z = jnp.sum(xg, axis=1, keepdims=True)
        gbuf[pl.ds(r, T), :] = jnp.broadcast_to(1.0 / (1.0 + jnp.exp(-z)), (T, T))

    c_all = c_ref[...]
    kk = _nn(c_all, wuk).astype(bf16)
    b_input()
    vv = _nn(c_all, wuv).astype(bf16)
    gate()
    qn = qproj(NB - 1)
    b_forward()
    mac_plan = {7: [15, 0], 6: [14, 1], 5: [13, 2], 4: [12, 3], 3: [11, 4], 2: [10, 5], 1: [9, 6], 0: [8, 7]}
    prev = None
    for i in range(NB - 1, -1, -1):
        w = (i + 1) * TQ
        q2 = qn
        sc = [scores(q2[:, h * D:(h + 1) * D], kk[0:w, h * D:(h + 1) * D]) for h in range(2)]
        b_mac(mac_plan[i][0])
        if i > 0:
            qn = qproj(i - 1)
        ctx0 = pv(sc[0], vv[0:w, 0:D])
        b_mac(mac_plan[i][1])
        if prev is not None:
            oproj(i + 1, prev)
        ctx1 = pv(sc[1], vv[0:w, D:2 * D])
        prev = jnp.concatenate([ctx0, ctx1], axis=1)
    oproj(0, prev)

    @pl.when(s == pl.num_programs(0) - 1)
    def _():
        def body(r, _):
            rows = pl.ds(pl.multiple_of(r * T, T), T)
            g = gbuf[rows, :]
            for j in range(M // T):
                a = acc[rows, j * T:(j + 1) * T]
                b = bbuf[j, rows, :]
                o_ref[rows, j * T:(j + 1) * T] = (b + g * (a - b)).astype(o_ref.dtype)
            return 0

        lax.fori_loop(0, S // T, body, 0)


@jax.jit
def pallas_gated_mix__compressed_kv_cla__ssm_conv_h3__prompt_kernel(
    A_x: jax.Array,
    A_c_kv: jax.Array,
    A_w_q: jax.Array,
    A_w_uk: jax.Array,
    A_w_uv: jax.Array,
    A_w_o: jax.Array,
    B_q: jax.Array,
    B_k: jax.Array,
    B_v: jax.Array,
    B_shift_k: jax.Array,
    B_ssm_k: jax.Array,
    B_ssm_D: jax.Array,
    gate_w: jax.Array,
):
    del B_q
    x = A_x.reshape(S, M)
    c = A_c_kv.reshape(S, C)
    bk = B_k.reshape(S, M)
    bv = B_v.reshape(S, M)
    sd = B_ssm_D.reshape(1, M)
    gw = gate_w.reshape(1, M)
    fwd, inv = _dft_tables()
    fwd = jnp.asarray(fwd, dtype=bf16)
    inv = jnp.asarray(inv, dtype=bf16)

    in_specs = [
        pl.BlockSpec((S, M), lambda s: (0, 0)),
        pl.BlockSpec((S, C), lambda s: (0, 0)),
        pl.BlockSpec((M, G, D), lambda s: (0, s // P, 0)),
        pl.BlockSpec((C, G, D), lambda s: (0, s // P, 0)),
        pl.BlockSpec((C, G, D), lambda s: (0, s // P, 0)),
        pl.BlockSpec((2, D, M), lambda s: (s, 0, 0)),
        pl.BlockSpec((S, T), lambda s: (0, s // 2)),
        pl.BlockSpec((S, T), lambda s: (0, s // 2)),
        pl.BlockSpec((S, T), lambda s: (0, s // 2)),
        pl.BlockSpec((T, KS), lambda s: (s // 2, 0)),
        pl.BlockSpec((T, S), lambda s: (s // 2, 0)),
        pl.BlockSpec((1, T), lambda s: (0, s // 2)),
        pl.BlockSpec((1, M), lambda s: (0, 0)),
        pl.BlockSpec((None, T, T), lambda s: (s % 2, 0, 0)),
        pl.BlockSpec((None, T, T), lambda s: (s % 2, 0, 0)),
    ]
    out = pl.pallas_call(
        _kernel,
        grid=(H // 2,),
        in_specs=in_specs,
        out_specs=pl.BlockSpec((S, M), lambda s: (0, 0)),
        out_shape=jax.ShapeDtypeStruct((S, M), bf16),
        scratch_shapes=[
            pltpu.VMEM((M * P, D), u32),
            pltpu.VMEM((C * P, D), u32),
            pltpu.VMEM((C * P, D), u32),
            pltpu.VMEM((S, M), f32),
            pltpu.VMEM((S + 8, T), f32),
            pltpu.VMEM((S, T), f32),
            pltpu.VMEM((M // T, S, T), f32),
            pltpu.VMEM((S, T), f32),
        ],
        compiler_params=pltpu.CompilerParams(
            dimension_semantics=("arbitrary",),
            vmem_limit_bytes=110 * 1024 * 1024,
        ),
        name="gated_mix",
    )(x, c, A_w_q, A_w_uk, A_w_uv, A_w_o, x, bk, bv, B_shift_k, B_ssm_k, sd, gw, fwd, inv)
    return out.reshape(1, S, M)
```

```python
import numpy as np
import jax
import jax.numpy as jnp
from jax import lax
import jax.experimental.pallas as pl
import jax.experimental.pallas.tpu as pltpu

OPTS = {}

S, M, H, D, C = 2048, 1024, 32, 128, 512
G = 8
P = G // 2
NG = H // G
NS = H // 2
T = 128
TQ = 256
NB = S // TQ
NC = S // T
NJ = M // T
KS = 4
SPLIT = 3
NEG = -1e9
QSCALE = float(D ** -0.5 * np.log2(np.e))
bf16 = jnp.bfloat16
f32 = jnp.float32
u32 = jnp.uint32

SEM_C = 0
NCC = 4
SEM_X = SEM_C + NCC
SEM_W = SEM_X + NB
SEM_WO = SEM_W + 3 * NG
SEM_B = SEM_WO + 3
SEM_S = SEM_B + 6
SEM_O = SEM_S + 5
NSEM = SEM_O + NB


def _nt(a, b):
    return lax.dot_general(a, b, (((1,), (1,)), ((), ())), preferred_element_type=f32)


def _nn(a, b):
    return jnp.dot(a, b, preferred_element_type=f32)


def _pack(v):
    return pltpu.bitcast(v, u32)


def _unpack(v):
    return pltpu.bitcast(v, bf16)


def _unpack_pair(w32):
    lo = lax.bitcast_convert_type(w32 << 16, f32).astype(bf16)
    hi = lax.bitcast_convert_type(w32 & u32(0xFFFF0000), f32).astype(bf16)
    return jnp.concatenate([lo, hi], axis=1)


def _recip(l):
    r = pl.reciprocal(l, approx=True)
    return r * (2.0 - l * r)


def _aligned(v, n):
    return v if isinstance(v, int) else pl.multiple_of(v, n)


def _dft_tables():
    n = np.arange(T)[None, :]
    k = np.arange(T)[:, None]
    ang = 2.0 * np.pi * ((n * (2 * k + 1)) % (4 * T)) / (4 * T)
    cos, sin = np.cos(ang), np.sin(ang)
    hf = T // 2
    halves = []
    for h in range(2):
        ks = np.arange(h * hf, (h + 1) * hf)
        ks = np.concatenate([ks[0::2], ks[1::2]])
        halves.append(np.concatenate([cos[ks], -sin[ks]], axis=0))
    fwd = np.stack(halves)
    inv = np.transpose(fwd, (0, 2, 1)) / T
    return fwd.astype(np.float32), inv.astype(np.float32)


def _kernel(x_hbm, c_hbm, wq_hbm, wuk_hbm, wuv_hbm, wo_hbm, bk_hbm, bv_hbm, sk_hbm,
            sh_hbm, sd_hbm, gw_hbm, f_hbm, gi_hbm,
            o_hbm,
            x_s, c_s, wq_b, wuk_b, wuv_b, wq32, wuk32, wuv32, wo_s, bk_s, bv_s, sk_s,
            sh_s, sd_s, gw_s, f_s, gi_s, par_s,
            kv32, qa32, qb32, cx32, bst, ut, osc,
            acc, kpad, ybuf, bbuf, gbuf, obuf, sems):
    def cp(src, dst, sem):
        return pltpu.make_async_copy(src, dst, sems.at[sem])

    def cp_c(i):
        r = pl.ds(i * (S // NCC), S // NCC)
        return cp(c_hbm.at[r, :], c_s.at[r, :], SEM_C + i)

    def cp_x(i):
        r = pl.ds(i * TQ, TQ)
        return cp(x_hbm.at[r, :], x_s.at[r, :], SEM_X + i)

    w_hbm = (wq_hbm, wuk_hbm, wuv_hbm)
    w_b = (wq_b, wuk_b, wuv_b)
    w_32 = (wq32, wuk32, wuv32)
    w_rows = (M, C, C)

    def cp_w(kind, g):
        return cp(w_hbm[kind].at[:, pl.ds(g * G, G), :], w_b[kind].at[g], SEM_W + kind * NG + g)

    def cp_wo(part):
        r = (pl.ds(0, 2), pl.ds(2, 2), pl.ds(4, H - 4))[part]
        return cp(wo_hbm.at[r], wo_s.at[r], SEM_WO + part)

    def cp_b(kind, part):
        r = (pl.ds(0, T), pl.ds(T, M - T))[part]
        if kind == 2:
            return cp(sk_hbm.at[r, :], sk_s.at[r, :], SEM_B + 2 * kind + part)
        src, dst = ((bk_hbm, bk_s), (bv_hbm, bv_s))[kind]
        return cp(src.at[:, r], dst.at[:, r], SEM_B + 2 * kind + part)

    def cp_small(i):
        src, dst = ((sh_hbm, sh_s), (sd_hbm, sd_s), (gw_hbm, gw_s), (f_hbm, f_s), (gi_hbm, gi_s))[i]
        return cp(src, dst, SEM_S + i)

    def cp_out(i):
        r = pl.ds(i * TQ, TQ if i <= SPLIT else (NB - SPLIT - 1) * TQ)
        return cp(obuf.at[r, :], o_hbm.at[r, :], SEM_O + i)

    def convert(kind, g_src, g_dst, r0, nrows):
        ch = 64
        for c0 in range(0, nrows, ch):
            v = w_b[kind][g_src, pl.ds(r0 + c0, ch), :, :]
            w_32[kind][g_dst, pl.ds((r0 + c0) * P, ch * P), :] = _pack(v.reshape(ch * G, D))

    def convert_loop(kind):
        def body(c, carry):
            convert(kind, 0, 0, pl.multiple_of(c * 64, 64), 64)
            return carry

        lax.fori_loop(0, w_rows[kind] // 64, body, 0)

    def load_w(kind, s):
        return _unpack_pair(w_32[kind][s // P, pl.ds(s % P, w_rows[kind], stride=P), :])

    row = lax.broadcasted_iota(jnp.int32, (T, T), 0)
    col = lax.broadcasted_iota(jnp.int32, (T, T), 1)
    hf = T // 2

    def kvproj(i, wuk, wuv):
        cc = c_s[i * TQ:(i + 1) * TQ, :]
        r = slice(i * TQ // 2, (i + 1) * TQ // 2)
        kv32[0, r, :] = _pack(_nn(cc, wuk).astype(bf16))
        kv32[1, r, :] = _pack(_nn(cc, wuv).astype(bf16))

    def qproj(i, wq):
        return (_nn(x_s[i * TQ:(i + 1) * TQ, :], wq) * QSCALE).astype(bf16)

    def scores(q, h, w):
        mask = col <= row
        k = _unpack(kv32[0, 0:w // 2, h * D:(h + 1) * D])
        s1 = _nt(q, k[0:w - T])
        s2 = _nt(q[T:], k[w - T:w])
        top_d = jnp.where(mask, s1[:T, w - 2 * T:], NEG)
        top = jnp.concatenate([s1[:T, :w - 2 * T], top_d], axis=1) if w > 2 * T else top_d
        bot = jnp.concatenate([s1[T:, :], jnp.where(mask, s2, NEG)], axis=1)
        return top, bot

    def softmax(sc):
        m = jnp.max(sc, axis=1, keepdims=True)
        p = jnp.exp2(sc - m)
        l = jnp.sum(p, axis=1, keepdims=True)
        return p.astype(bf16), l

    def pv(sc, h, w):
        top, bot = sc
        v = _unpack(kv32[1, 0:w // 2, h * D:(h + 1) * D])
        if OPTS.get("pk", "1") == "0":
            pt, lt = softmax(top)
            pb, lb = softmax(bot)
            p1 = jnp.concatenate([pt, pb[:, :w - T]], axis=0)
            o1 = _nn(p1, v[0:w - T])
            o2 = _nn(pb[:, w - T:], v[w - T:w])
            ot = o1[:T] * _recip(lt)
            ob = (o1[T:] + o2) * _recip(lb)
            return jnp.concatenate([ot, ob], axis=0).astype(bf16)
        pt = jnp.exp2(top - jnp.max(top, axis=1, keepdims=True))
        pb = jnp.exp2(bot - jnp.max(bot, axis=1, keepdims=True))
        pk = pltpu.pack_elementwise([pt, pb[:, :w - T]], packed_dtype=bf16)
        pl_ = pb[:, w - T:].astype(bf16)
        o1 = _nn(_unpack(pk), v[0:w - T])
        o2 = _nn(pl_, v[w - T:w])
        lo = pltpu.unpack_elementwise(pk, index=0, packed_dtype=bf16, unpacked_dtype=f32)
        hi = pltpu.unpack_elementwise(pk, index=1, packed_dtype=bf16, unpacked_dtype=f32)
        lt = jnp.sum(lo, axis=1, keepdims=True)
        lb = jnp.sum(jnp.concatenate([hi, pl_.astype(f32)], axis=1), axis=1, keepdims=True)
        osc[h] = o1
        ot = osc[h, pl.ds(0, T, stride=2), :] * _recip(lt)
        ob = (osc[h, pl.ds(1, T, stride=2), :] + o2) * _recip(lb)
        return jnp.concatenate([ot, ob], axis=0).astype(bf16)

    def combine(i, a):
        rows = slice(i * TQ, (i + 1) * TQ)
        g = gbuf[rows, :]
        for jj in range(NJ):
            b = bbuf[jj, rows, :]
            obuf[rows, jj * T:(jj + 1) * T] = (b + g * (a[:, jj * T:(jj + 1) * T] - b)).astype(bf16)

    def oproj(i, ctx2, wo, final=False):
        rows = slice(i * TQ, (i + 1) * TQ)
        a = _nn(ctx2, wo) + acc[rows, :]
        if final:
            combine(i, a)
        else:
            acc[rows, :] = a

    def load_wo(s):
        return wo_s[pl.ds(2 * s, 2)].reshape(2 * D, M)

    def b_piece(s, a, prev_h):
        j = s // 2
        jl = pl.ds(_aligned(j * T, T), T)
        rows = slice(a * T, (a + 1) * T)
        taps = par_s[pl.ds(_aligned(j * 8, 8), 8), :]
        kf = bk_s[rows, jl].astype(f32)
        kpad[8 + a * T:8 + (a + 1) * T, :] = kf
        ks = kf * taps[0:1, :]
        for t in range(1, KS):
            ks = ks + kpad[8 - t + a * T:8 - t + (a + 1) * T, :] * taps[t:t + 1, :]
        u = ks * bv_s[rows, jl].astype(f32)
        ut[rows, :] = u * taps[KS:KS + 1, :]
        fm = f_s[s % 2]
        uh = _nn(fm, u.astype(bf16))
        ur, ui = uh[0:hf], uh[hf:T]
        bst[0, a] = ur
        bst[1, a] = ui
        bst[2, a] = ur + ui
        hh = _nt(fm, sk_s[pl.ds(_aligned(j * T, T), T), rows])
        hr, hi = hh[0:hf], hh[hf:T]
        if prev_h is not None:
            pr, pi = prev_h[0:hf], prev_h[hf:T]
            q = hf // 2
            hr = jnp.concatenate([hr[:q] - pi[:q], hr[q:] + pi[q:]], axis=0)
            hi = jnp.concatenate([hi[:q] + pr[:q], hi[q:] - pr[q:]], axis=0)
        bst[3, a] = hr
        bst[4, a] = hi - hr
        bst[5, a] = hr + hi
        return hh

    def b_front(s):
        ph = None
        for a in range(NC):
            ph = b_piece(s, a, ph)

    def b_mac(s, c, last=False):
        k1 = k2 = k3 = None
        for a in range(c + 1):
            jj = c - a
            t1 = bst[3, jj] * bst[2, a]
            t2 = bst[0, a] * bst[4, jj]
            t3 = bst[1, a] * bst[5, jj]
            k1 = t1 if k1 is None else k1 + t1
            k2 = t2 if k2 is None else k2 + t2
            k3 = t3 if k3 is None else k3 + t3
        z = jnp.concatenate([k1 - k3, k1 + k2], axis=0).astype(bf16)
        rows = slice(c * T, (c + 1) * T)
        y = _nn(gi_s[s % 2], z)
        if last:
            y = y + ybuf[rows, :]
        else:
            y = y + jnp.where(s % 2 == 1, ybuf[rows, :], 0.0)
            ybuf[rows, :] = y
        j = s // 2
        jl = pl.ds(_aligned(j * T, T), T)
        bbuf[j, rows, :] = x_s[rows, jl].astype(f32) * (y + ut[rows, :])

    def gate(s):
        r = pl.ds(_aligned(S - T - s * T, T), T)
        xg = x_s[r, :].astype(f32) * gw_s[...].astype(f32).reshape(1, M)
        z = jnp.sum(xg, axis=1, keepdims=True)
        gbuf[r, :] = jnp.broadcast_to(1.0 / (1.0 + jnp.exp(-z)), (T, T))

    def front_first():
        cp_w(1, 0).start()
        cp_w(2, 0).start()
        for i in range(NCC):
            cp_c(i).start()
        cp_w(0, 0).start()
        cp_x(NB - 1).start()
        for i in range(5):
            cp_small(i).start()
        for kind in range(3):
            cp_b(kind, 0).start()
        for i in range(NB - 2, 1, -1):
            cp_x(i).start()
        cp_wo(0).start()
        cp_x(1).start()
        cp_x(0).start()
        kpad[0:8, :] = jnp.zeros((8, T), f32)

        def zero(i, carry):
            acc[pl.ds(pl.multiple_of(i * 64, 64), 64), :] = jnp.zeros((64, M), f32)
            return carry

        lax.fori_loop(0, S // 64, zero, 0)
        cp_w(1, 0).wait()
        convert_loop(1)
        cp_w(2, 0).wait()
        convert_loop(2)
        rc = S // NCC

        def kv_chunk(i, carry):
            r = pl.ds(pl.multiple_of(i * rc, rc), rc)
            pltpu.make_async_copy(c_hbm.at[r, :], c_s.at[r, :], sems.at[SEM_C + i]).wait()
            cc = c_s[r, :]
            rp = pl.ds(pl.multiple_of(i * (rc // 2), rc // 2), rc // 2)
            kv32[0, rp, :] = _pack(_nn(cc, load_w(1, 0)).astype(bf16))
            kv32[1, rp, :] = _pack(_nn(cc, load_w(2, 0)).astype(bf16))
            return carry

        lax.fori_loop(0, NCC, kv_chunk, 0)
        cp_w(0, 0).wait()
        convert_loop(0)
        cp_x(NB - 1).wait()
        qa32[...] = _pack(qproj(NB - 1, load_w(0, 0)))
        for i in range(5):
            cp_small(i).wait()
        for kind in range(3):
            cp_b(kind, 0).wait()
        shf = sh_s[...].astype(f32)
        sdf = sd_s[...].astype(f32).reshape(1, M)
        for jj in range(NJ):
            par_s[jj * 8:jj * 8 + KS, :] = shf[:, jj * T:(jj + 1) * T]
            par_s[jj * 8 + KS:jj * 8 + KS + 1, :] = sdf[:, jj * T:(jj + 1) * T]
            par_s[jj * 8 + KS + 1:jj * 8 + 8, :] = jnp.zeros((8 - KS - 1, T), f32)
        b_front(0)
        gate(0)
        for i in range(NB - 2, 1, -1):
            cp_x(i).wait()
        cp_wo(0).wait()
        cp_wo(1).start()
        for kind in range(3):
            cp_w(kind, 1).start()

    mac_a = {7: [15, 4], 6: [14, 5], 5: [13, 6], 4: [12, 7, 8], 3: [11, 10, 9]}

    def seg_a(s):
        wq = load_w(0, s)
        wo = load_wo(s)
        qn = _unpack(qa32[...])
        prev = None
        order = OPTS.get("oa", "SA.SB.Q.M0.PA.O.M1.PB").split(".")
        for i in range(NB - 1, SPLIT - 1, -1):
            w = (i + 1) * TQ
            q2 = qn
            sc = [None, None]
            ctx = [None, None]
            for op in order:
                if op == "SA":
                    sc[0] = scores(q2[:, 0:D], 0, w)
                elif op == "SB":
                    sc[1] = scores(q2[:, D:2 * D], 1, w)
                elif op == "M0":
                    b_mac(s, mac_a[i][0])
                elif op == "M1":
                    for c in mac_a[i][1:]:
                        b_mac(s, c)
                elif op == "Q":
                    qn = qproj(i - 1, wq)
                elif op == "PA":
                    ctx[0] = pv(sc[0], 0, w)
                elif op == "PB":
                    ctx[1] = pv(sc[1], 1, w)
                elif op == "O":
                    if prev is not None:
                        oproj(i + 1, prev, wo)
            prev = jnp.concatenate(ctx, axis=1)
        qb32[...] = _pack(qn)
        cx32[...] = _pack(prev)

    def seg_b(s, last):
        if not last:
            sn = s + 1
            gsrc = jnp.minimum(s // P + 1, NG - 1)
            gdst = s // P + 1
            q4 = s % P
            for kind in range(3):
                n = w_rows[kind] // P
                convert(kind, gsrc, gdst, _aligned(q4 * n, n), n)
            wuk = load_w(1, sn)
            wuv = load_w(2, sn)
        wq = load_w(0, s)
        wo = load_wo(s)
        st = {"q": _unpack(qb32[...]), "prev": _unpack(cx32[...]), "h": None, "a": 0}

        def job(name):
            kind, i = name[0], int(name[-1])
            if name[0] == "M":
                b_mac(s, i, last)
            elif name[:2] in ("SA", "SB"):
                h = 0 if name[1] == "A" else 1
                st["sc", h] = scores(st["q", i][:, h * D:(h + 1) * D], h, (i + 1) * TQ)
            elif kind == "Q":
                st["q", i] = qproj(i, wq)
            elif name[:2] in ("PA", "PB"):
                h = 0 if name[1] == "A" else 1
                st["ctx", i, h] = pv(st["sc", h], h, (i + 1) * TQ)
            elif kind == "O":
                ctx = st["prev"] if i == SPLIT else jnp.concatenate([st["ctx", i, 0], st["ctx", i, 1]], axis=1)
                oproj(i, ctx, wo, last)
            elif kind == "K":
                if not last:
                    kvproj(i, wuk, wuv)
            elif kind == "N":
                if not last:
                    qa32[...] = _pack(qproj(NB - 1, load_w(0, sn)))
            elif kind == "G":
                if not last:
                    gate(sn)
            elif kind == "C":
                if last:
                    combine(i, acc[i * TQ:(i + 1) * TQ, :])
            elif kind == "D":
                if last:
                    cp_out(i).start()
            elif kind == "F":
                if not last:
                    for _ in range(i):
                        if st["a"] < NC:
                            st["h"] = b_piece(sn, st["a"], st["h"])
                            st["a"] += 1

        st["q", SPLIT - 1] = st["q"]
        jobs = OPTS.get("ob", "M3.M2.M1.M0.SA2.SB2.F1.Q1.F1.PA2.F1.O3.F1.K7.F1.PB2.F1.K6.F1.SA1.SB1.F1.Q0.F1.PA1.F1.O2.F1."
                        "K5.F1.PB1.K4.F1.K2.F1.SA0.SB0.K3.F1.PA0.O1.F1.PB0.G0.K1.O0.K0.N0").split(".")
        if last:
            jobs = OPTS.get("ol", "M3.M2.M1.M0.SA2.C7.SB2.C6.Q1.C5.C4.D4.PA2.O3.D3.PB2.SA1.SB1.Q0.PA1.O2.D2.PB1.SA0.SB0.PA0.O1.D1.PB0.O0.D0").split(".")
        for name in jobs:
            job(name)
        if not last:
            assert st["a"] == NC, st["a"]
        else:
            for i in range(SPLIT + 2):
                cp_out(i).wait()


    front_first()

    def step(s, carry):
        seg_a(s)

        @pl.when(s == 0)
        def _():
            cp_x(1).wait()
            cp_x(0).wait()
            cp_wo(1).wait()
            for kind in range(3):
                cp_w(kind, 1).wait()
            for kind in range(3):
                cp_b(kind, 1).start()
            cp_wo(2).start()
            for g in range(2, NG):
                for kind in range(3):
                    cp_w(kind, g).start()

        @pl.when(s == 1)
        def _():
            cp_wo(2).wait()
            for kind in range(3):
                cp_b(kind, 1).wait()

        for g in range(2, NG):
            @pl.when(s == (g - 1) * P)
            def _():
                for kind in range(3):
                    cp_w(kind, g).wait()

        @pl.when(s < NS - 1)
        def _():
            seg_b(s, False)

        @pl.when(s == NS - 1)
        def _():
            seg_b(s, True)

        return carry

    lax.fori_loop(0, NS, step, 0)


@jax.jit
def pallas_gated_mix__compressed_kv_cla__ssm_conv_h3__prompt_kernel(
    A_x: jax.Array,
    A_c_kv: jax.Array,
    A_w_q: jax.Array,
    A_w_uk: jax.Array,
    A_w_uv: jax.Array,
    A_w_o: jax.Array,
    B_q: jax.Array,
    B_k: jax.Array,
    B_v: jax.Array,
    B_shift_k: jax.Array,
    B_ssm_k: jax.Array,
    B_ssm_D: jax.Array,
    gate_w: jax.Array,
):
    del B_q
    x = A_x.reshape(S, M)
    c = A_c_kv.reshape(S, C)
    bk = B_k.reshape(S, M)
    bv = B_v.reshape(S, M)
    sh = B_shift_k.T
    fwd, inv = _dft_tables()
    fwd = jnp.asarray(fwd, dtype=bf16)
    inv = jnp.asarray(inv, dtype=bf16)

    any_spec = pl.BlockSpec(memory_space=pl.ANY)
    out = pl.pallas_call(
        _kernel,
        in_specs=[any_spec] * 14,
        out_specs=any_spec,
        out_shape=jax.ShapeDtypeStruct((S, M), bf16),
        scratch_shapes=[
            pltpu.VMEM((S, M), bf16),
            pltpu.VMEM((S, C), bf16),
            pltpu.VMEM((NG, M, G, D), bf16),
            pltpu.VMEM((NG, C, G, D), bf16),
            pltpu.VMEM((NG, C, G, D), bf16),
            pltpu.VMEM((NG + 1, M * P, D), u32),
            pltpu.VMEM((NG + 1, C * P, D), u32),
            pltpu.VMEM((NG + 1, C * P, D), u32),
            pltpu.VMEM((H, D, M), bf16),
            pltpu.VMEM((S, M), bf16),
            pltpu.VMEM((S, M), bf16),
            pltpu.VMEM((M, S), bf16),
            pltpu.VMEM((KS, M), bf16),
            pltpu.VMEM((M,), bf16),
            pltpu.VMEM((M,), bf16),
            pltpu.VMEM((2, T, T), bf16),
            pltpu.VMEM((2, T, T), bf16),
            pltpu.VMEM((NJ * 8, T), f32),
            pltpu.VMEM((2, S // 2, 2 * D), u32),
            pltpu.VMEM((TQ // 2, 2 * D), u32),
            pltpu.VMEM((TQ // 2, 2 * D), u32),
            pltpu.VMEM((TQ // 2, 2 * D), u32),
            pltpu.VMEM((6, NC, T // 2, T), f32),
            pltpu.VMEM((S, T), f32),
            pltpu.VMEM((2, TQ, D), f32),
            pltpu.VMEM((S, M), f32),
            pltpu.VMEM((S + 8, T), f32),
            pltpu.VMEM((S, T), f32),
            pltpu.VMEM((NJ, S, T), f32),
            pltpu.VMEM((S, T), f32),
            pltpu.VMEM((S, M), bf16),
            pltpu.SemaphoreType.DMA((NSEM,)),
        ],
        compiler_params=pltpu.CompilerParams(
            vmem_limit_bytes=120 * 1024 * 1024,
            shape_invariant_numerics=(OPTS.get("sin", "1") == "1"),
        ),
        name="gated_mix",
    )(x, c, A_w_q, A_w_uk, A_w_uv, A_w_o, bk, bv, B_ssm_k, sh, B_ssm_D, gate_w, fwd, inv)
    return out.reshape(1, S, M)
```

```python
import numpy as np
import jax
import jax.numpy as jnp
from jax import lax
import jax.experimental.pallas as pl
import jax.experimental.pallas.tpu as pltpu

OPTS = {}

S, M, H, D, C = 2048, 1024, 32, 128, 512
G = 8
P = G // 2
NG = H // G
NS = H // 2
T = 128
TQ = 256
NB = S // TQ
NC = S // T
NJ = M // T
KS = 4
SPLIT = 3
NEG = -1e9
QSCALE = float(D ** -0.5 * np.log2(np.e))
bf16 = jnp.bfloat16
f32 = jnp.float32
u32 = jnp.uint32

SEM_C = 0
NCC = 4
SEM_X = SEM_C + NCC
SEM_W = SEM_X + NB
SEM_WO = SEM_W + 3 * NG
SEM_B = SEM_WO + 3
SEM_S = SEM_B + 6
SEM_O = SEM_S + 5
NSEM = SEM_O + NB


def _nt(a, b):
    return lax.dot_general(a, b, (((1,), (1,)), ((), ())), preferred_element_type=f32)


def _nn(a, b):
    return jnp.dot(a, b, preferred_element_type=f32)


def _pack(v):
    return pltpu.bitcast(v, u32)


def _unpack(v):
    return pltpu.bitcast(v, bf16)


def _unpack_pair(w32):
    lo = lax.bitcast_convert_type(w32 << 16, f32).astype(bf16)
    hi = lax.bitcast_convert_type(w32 & u32(0xFFFF0000), f32).astype(bf16)
    return jnp.concatenate([lo, hi], axis=1)


def _recip(l):
    r = pl.reciprocal(l, approx=True)
    return r * (2.0 - l * r)


def _aligned(v, n):
    return v if isinstance(v, int) else pl.multiple_of(v, n)


def _dft_tables():
    n = np.arange(T)[None, :]
    k = np.arange(T)[:, None]
    ang = 2.0 * np.pi * ((n * (2 * k + 1)) % (4 * T)) / (4 * T)
    cos, sin = np.cos(ang), np.sin(ang)
    hf = T // 2
    halves = []
    for h in range(2):
        ks = np.arange(h * hf, (h + 1) * hf)
        ks = np.concatenate([ks[0::2], ks[1::2]])
        halves.append(np.concatenate([cos[ks], -sin[ks]], axis=0))
    fwd = np.stack(halves)
    inv = np.transpose(fwd, (0, 2, 1)) / T
    return fwd.astype(np.float32), inv.astype(np.float32)


def _kernel(x_hbm, c_hbm, wq_hbm, wuk_hbm, wuv_hbm, wo_hbm, bk_hbm, bv_hbm, sk_hbm,
            sh_hbm, sd_hbm, gw_hbm, f_hbm, gi_hbm,
            o_hbm,
            x_s, c_s, wq_b, wuk_b, wuv_b, wq32, wuk32, wuv32, wo_s, bk_s, bv_s, sk_s,
            sh_s, sd_s, gw_s, f_s, gi_s, par_s,
            kv32, qa32, qb32, cx32, bst, ut, osc, x32, c32,
            acc, kpad, ybuf, bbuf, gbuf, obuf, sems):
    def cp(src, dst, sem):
        return pltpu.make_async_copy(src, dst, sems.at[sem])

    def cp_c(i):
        r = pl.ds(i * (S // NCC), S // NCC)
        return cp(c_hbm.at[r, :], c_s.at[r, :], SEM_C + i)

    def cp_x(i):
        r = pl.ds(i * TQ, TQ)
        return cp(x_hbm.at[r, :], x_s.at[r, :], SEM_X + i)

    w_hbm = (wq_hbm, wuk_hbm, wuv_hbm)
    w_b = (wq_b, wuk_b, wuv_b)
    w_32 = (wq32, wuk32, wuv32)
    w_rows = (M, C, C)

    def cp_w(kind, g):
        return cp(w_hbm[kind].at[:, pl.ds(g * G, G), :], w_b[kind].at[g], SEM_W + kind * NG + g)

    def cp_wo(part):
        r = (pl.ds(0, 2), pl.ds(2, 2), pl.ds(4, H - 4))[part]
        return cp(wo_hbm.at[r], wo_s.at[r], SEM_WO + part)

    def cp_b(kind, part):
        r = (pl.ds(0, T), pl.ds(T, M - T))[part]
        if kind == 2:
            return cp(sk_hbm.at[r, :], sk_s.at[r, :], SEM_B + 2 * kind + part)
        src, dst = ((bk_hbm, bk_s), (bv_hbm, bv_s))[kind]
        return cp(src.at[:, r], dst.at[:, r], SEM_B + 2 * kind + part)

    def cp_small(i):
        src, dst = ((sh_hbm, sh_s), (sd_hbm, sd_s), (gw_hbm, gw_s), (f_hbm, f_s), (gi_hbm, gi_s))[i]
        return cp(src, dst, SEM_S + i)

    def cp_out(i):
        r = pl.ds(i * TQ, TQ if i <= SPLIT else (NB - SPLIT - 1) * TQ)
        return cp(obuf.at[r, :], o_hbm.at[r, :], SEM_O + i)

    def convert(kind, g_src, g_dst, r0, nrows):
        ch = 64
        for c0 in range(0, nrows, ch):
            v = w_b[kind][g_src, pl.ds(r0 + c0, ch), :, :]
            w_32[kind][g_dst, pl.ds((r0 + c0) * P, ch * P), :] = _pack(v.reshape(ch * G, D))

    def convert_loop(kind):
        def body(c, carry):
            convert(kind, 0, 0, pl.multiple_of(c * 64, 64), 64)
            return carry

        lax.fori_loop(0, w_rows[kind] // 64, body, 0)

    def pack_x(i):
        def body(c, carry):
            r = pl.multiple_of(i * TQ + c * 64, 64)
            x32[pl.ds(pl.multiple_of(r // 2, 32), 32), :] = _pack(x_s[pl.ds(r, 64), :])
            return carry

        lax.fori_loop(0, TQ // 64, body, 0)

    def load_w(kind, s):
        return _unpack_pair(w_32[kind][s // P, pl.ds(s % P, w_rows[kind], stride=P), :])

    row = lax.broadcasted_iota(jnp.int32, (T, T), 0)
    col = lax.broadcasted_iota(jnp.int32, (T, T), 1)
    hf = T // 2

    def kvproj(i, wuk, wuv):
        cc = _unpack(c32[i * TQ // 2:(i + 1) * TQ // 2, :])
        r = slice(i * TQ // 2, (i + 1) * TQ // 2)
        kv32[0, r, :] = _pack(_nn(cc, wuk).astype(bf16))
        kv32[1, r, :] = _pack(_nn(cc, wuv).astype(bf16))

    def qproj(i, wq):
        return (_nn(_unpack(x32[i * TQ // 2:(i + 1) * TQ // 2, :]), wq) * QSCALE).astype(bf16)

    def scores(q, h, w):
        mask = col <= row
        k = _unpack(kv32[0, 0:w // 2, h * D:(h + 1) * D])
        s1 = _nt(q, k[0:w - T])
        s2 = _nt(q[T:], k[w - T:w])
        top_d = jnp.where(mask, s1[:T, w - 2 * T:], NEG)
        top = jnp.concatenate([s1[:T, :w - 2 * T], top_d], axis=1) if w > 2 * T else top_d
        bot = jnp.concatenate([s1[T:, :], jnp.where(mask, s2, NEG)], axis=1)
        return top, bot

    def softmax(sc):
        m = jnp.max(sc, axis=1, keepdims=True)
        p = jnp.exp2(sc - m)
        l = jnp.sum(p, axis=1, keepdims=True)
        return p.astype(bf16), l

    def pv(sc, h, w):
        top, bot = sc
        v = _unpack(kv32[1, 0:w // 2, h * D:(h + 1) * D])
        if OPTS.get("pk", "1") == "0":
            pt, lt = softmax(top)
            pb, lb = softmax(bot)
            p1 = jnp.concatenate([pt, pb[:, :w - T]], axis=0)
            o1 = _nn(p1, v[0:w - T])
            o2 = _nn(pb[:, w - T:], v[w - T:w])
            ot = o1[:T] * _recip(lt)
            ob = (o1[T:] + o2) * _recip(lb)
            return jnp.concatenate([ot, ob], axis=0).astype(bf16)
        pt = jnp.exp2(top - jnp.max(top, axis=1, keepdims=True))
        pb = jnp.exp2(bot - jnp.max(bot, axis=1, keepdims=True))
        pk = pltpu.pack_elementwise([pt, pb[:, :w - T]], packed_dtype=bf16)
        pl_ = pb[:, w - T:].astype(bf16)
        o1 = _nn(_unpack(pk), v[0:w - T])
        o2 = _nn(pl_, v[w - T:w])
        lo = pltpu.unpack_elementwise(pk, index=0, packed_dtype=bf16, unpacked_dtype=f32)
        hi = pltpu.unpack_elementwise(pk, index=1, packed_dtype=bf16, unpacked_dtype=f32)
        lt = jnp.sum(lo, axis=1, keepdims=True)
        lb = jnp.sum(jnp.concatenate([hi, pl_.astype(f32)], axis=1), axis=1, keepdims=True)
        osc[h] = o1
        ot = osc[h, pl.ds(0, T, stride=2), :] * _recip(lt)
        ob = (osc[h, pl.ds(1, T, stride=2), :] + o2) * _recip(lb)
        return jnp.concatenate([ot, ob], axis=0).astype(bf16)

    def combine(i, a):
        rows = slice(i * TQ, (i + 1) * TQ)
        g = gbuf[rows, :]
        for jj in range(NJ):
            b = bbuf[jj, rows, :]
            obuf[rows, jj * T:(jj + 1) * T] = (b + g * (a[:, jj * T:(jj + 1) * T] - b)).astype(bf16)

    def oproj(i, ctx2, wo, final=False):
        rows = slice(i * TQ, (i + 1) * TQ)
        a = _nn(ctx2, wo) + acc[rows, :]
        if final:
            combine(i, a)
        else:
            acc[rows, :] = a

    def load_wo(s):
        return wo_s[pl.ds(2 * s, 2)].reshape(2 * D, M)

    def b_piece(s, a, prev, anchor=None):
        j = s // 2
        jl = pl.ds(_aligned(j * T, T), T)
        rows = slice(a * T, (a + 1) * T)
        taps = par_s[pl.ds(_aligned(j * 8, 8), 8), :]
        if anchor is not None:
            taps = taps + anchor * 0.0
        kf = bk_s[rows, jl].astype(f32)
        ks = kf * taps[0:1, :]
        if OPTS.get("fir", "roll") == "roll":
            tail = prev[1] if prev is not None else jnp.zeros((8, T), f32)
            ext = jnp.concatenate([tail, kf], axis=0)
            for t in range(1, KS):
                ks = ks + pltpu.roll(ext, t, 0)[8:, :] * taps[t:t + 1, :]
        else:
            kpad[8 + a * T:8 + (a + 1) * T, :] = kf
            for t in range(1, KS):
                ks = ks + kpad[8 - t + a * T:8 - t + (a + 1) * T, :] * taps[t:t + 1, :]
        u = ks * bv_s[rows, jl].astype(f32)
        ut[rows, :] = u * taps[KS:KS + 1, :]
        fm = f_s[s % 2]
        uh = _nn(fm, u.astype(bf16))
        ur, ui = uh[0:hf], uh[hf:T]
        bst[0, a] = ur
        bst[1, a] = ui
        bst[2, a] = ur + ui
        hh = _nt(fm, sk_s[pl.ds(_aligned(j * T, T), T), rows])
        hr, hi = hh[0:hf], hh[hf:T]
        if prev is not None:
            prev_h = prev[0]
            pr, pi = prev_h[0:hf], prev_h[hf:T]
            q = hf // 2
            hr = jnp.concatenate([hr[:q] - pi[:q], hr[q:] + pi[q:]], axis=0)
            hi = jnp.concatenate([hi[:q] + pr[:q], hi[q:] - pr[q:]], axis=0)
        bst[3, a] = hr
        bst[4, a] = hi - hr
        bst[5, a] = hr + hi
        return hh, kf[T - 8:, :]

    def b_front(s):
        ph = None
        for a in range(NC):
            ph = b_piece(s, a, ph)

    def b_mac(s, c, last=False):
        k1 = k2 = k3 = None
        for a in range(c + 1):
            jj = c - a
            t1 = bst[3, jj] * bst[2, a]
            t2 = bst[0, a] * bst[4, jj]
            t3 = bst[1, a] * bst[5, jj]
            k1 = t1 if k1 is None else k1 + t1
            k2 = t2 if k2 is None else k2 + t2
            k3 = t3 if k3 is None else k3 + t3
        z = jnp.concatenate([k1 - k3, k1 + k2], axis=0).astype(bf16)
        rows = slice(c * T, (c + 1) * T)
        y = _nn(gi_s[s % 2], z)
        if last:
            y = y + ybuf[rows, :]
        else:
            y = y + jnp.where(s % 2 == 1, ybuf[rows, :], 0.0)
            ybuf[rows, :] = y
        j = s // 2
        jl = pl.ds(_aligned(j * T, T), T)
        bbuf[j, rows, :] = x_s[rows, jl].astype(f32) * (y + ut[rows, :])

    def gate(s):
        r = pl.ds(_aligned(S - T - s * T, T), T)
        xg = x_s[r, :].astype(f32) * gw_s[...].astype(f32).reshape(1, M)
        z = jnp.sum(xg, axis=1, keepdims=True)
        g = jnp.broadcast_to(1.0 / (1.0 + jnp.exp(-z)), (T, T))
        gbuf[r, :] = g
        return jnp.max(g.reshape(T // 8, 8, T), axis=0)

    def front_first():
        cp_w(1, 0).start()
        cp_w(2, 0).start()
        for i in range(NCC):
            cp_c(i).start()
        cp_w(0, 0).start()
        cp_x(NB - 1).start()
        for i in range(5):
            cp_small(i).start()
        for kind in range(3):
            cp_b(kind, 0).start()
        for i in range(NB - 2, 1, -1):
            cp_x(i).start()
        cp_wo(0).start()
        cp_x(1).start()
        cp_x(0).start()
        kpad[0:8, :] = jnp.zeros((8, T), f32)

        def zero(i, carry):
            acc[pl.ds(pl.multiple_of(i * 64, 64), 64), :] = jnp.zeros((64, M), f32)
            return carry

        lax.fori_loop(0, S // 64, zero, 0)
        cp_w(1, 0).wait()
        convert_loop(1)
        cp_w(2, 0).wait()
        convert_loop(2)
        rc = S // NCC

        def kv_chunk(i, carry):
            r = pl.ds(pl.multiple_of(i * rc, rc), rc)
            pltpu.make_async_copy(c_hbm.at[r, :], c_s.at[r, :], sems.at[SEM_C + i]).wait()
            cc = c_s[r, :]
            rp = pl.ds(pl.multiple_of(i * (rc // 2), rc // 2), rc // 2)
            c32[rp, :] = _pack(cc)
            kv32[0, rp, :] = _pack(_nn(cc, load_w(1, 0)).astype(bf16))
            kv32[1, rp, :] = _pack(_nn(cc, load_w(2, 0)).astype(bf16))
            return carry

        lax.fori_loop(0, NCC, kv_chunk, 0)
        cp_w(0, 0).wait()
        convert_loop(0)
        cp_x(NB - 1).wait()
        pack_x(NB - 1)
        qa32[...] = _pack(qproj(NB - 1, load_w(0, 0)))
        for i in range(5):
            cp_small(i).wait()
        for kind in range(3):
            cp_b(kind, 0).wait()
        shf = sh_s[...].astype(f32)
        sdf = sd_s[...].astype(f32).reshape(1, M)
        for jj in range(NJ):
            par_s[jj * 8:jj * 8 + KS, :] = shf[:, jj * T:(jj + 1) * T]
            par_s[jj * 8 + KS:jj * 8 + KS + 1, :] = sdf[:, jj * T:(jj + 1) * T]
            par_s[jj * 8 + KS + 1:jj * 8 + 8, :] = jnp.zeros((8 - KS - 1, T), f32)
        b_front(0)
        gate(0)
        for i in range(NB - 2, 1, -1):
            cp_x(i).wait()
            pack_x(i)
        cp_wo(0).wait()
        cp_wo(1).start()
        for kind in range(3):
            cp_w(kind, 1).start()

    mac_a = {7: [15, 4], 6: [14, 5], 5: [13, 6], 4: [12, 7, 8], 3: [11, 10, 9]}
    if "mp" in OPTS:
        mac_a = {7 - n: [int(c) for c in grp.split("-") if c] for n, grp in enumerate(OPTS["mp"].split("_"))}
        assert sorted(sum(mac_a.values(), [])) == list(range(4, 16))

    def seg_a(s):
        wq = load_w(0, s)
        wo = load_wo(s)
        qn = _unpack(qa32[...])
        prev = None
        for i in range(NB - 1, SPLIT - 1, -1):
            order = OPTS.get("oa", "SA.SB.Q.M0.PA.O.M1.PB").split(".")
            if i == SPLIT and "oa3" in OPTS:
                order = OPTS["oa3"].split(".")
            w = (i + 1) * TQ
            q2 = qn
            sc = [None, None]
            ctx = [None, None]
            for op in order:
                if op == "SA":
                    sc[0] = scores(q2[:, 0:D], 0, w)
                elif op == "SB":
                    sc[1] = scores(q2[:, D:2 * D], 1, w)
                elif op == "M0":
                    for c in mac_a[i][:1]:
                        b_mac(s, c)
                elif op == "M1":
                    for c in mac_a[i][1:]:
                        b_mac(s, c)
                elif op == "Q":
                    qn = qproj(i - 1, wq)
                elif op == "PA":
                    ctx[0] = pv(sc[0], 0, w)
                elif op == "PB":
                    ctx[1] = pv(sc[1], 1, w)
                elif op == "O":
                    if prev is not None:
                        oproj(i + 1, prev, wo)
            prev = jnp.concatenate(ctx, axis=1)
        qb32[...] = _pack(qn)
        cx32[...] = _pack(prev)

    def seg_b(s, last):
        if not last:
            sn = s + 1
            gsrc = jnp.minimum(s // P + 1, NG - 1)
            gdst = s // P + 1
            q4 = s % P
            for kind in range(3):
                n = w_rows[kind] // P
                convert(kind, gsrc, gdst, _aligned(q4 * n, n), n)
            wuk = load_w(1, sn)
            wuv = load_w(2, sn)
        wq = load_w(0, s)
        wo = load_wo(s)
        st = {"q": _unpack(qb32[...]), "prev": _unpack(cx32[...]), "h": None, "a": 0}

        def job(name):
            kind, i = name[0], int(name[-1])
            if name[0] == "M":
                b_mac(s, i, last)
            elif name[:2] in ("SA", "SB"):
                h = 0 if name[1] == "A" else 1
                st["sc", h] = scores(st["q", i][:, h * D:(h + 1) * D], h, (i + 1) * TQ)
            elif kind == "Q":
                st["q", i] = qproj(i, wq)
            elif name[:2] in ("PA", "PB"):
                h = 0 if name[1] == "A" else 1
                st["ctx", i, h] = pv(st["sc", h], h, (i + 1) * TQ)
            elif kind == "O":
                ctx = st["prev"] if i == SPLIT else jnp.concatenate([st["ctx", i, 0], st["ctx", i, 1]], axis=1)
                oproj(i, ctx, wo, last)
            elif kind == "K":
                if not last:
                    kvproj(i, wuk, wuv)
            elif kind == "N":
                if not last:
                    qa32[...] = _pack(qproj(NB - 1, load_w(0, sn)))
            elif kind == "G":
                if not last:
                    g8 = gate(sn)
                    if OPTS.get("ga", "0") == "1":
                        st["anchor"] = g8
            elif kind == "C":
                if last:
                    combine(i, acc[i * TQ:(i + 1) * TQ, :])
            elif kind == "D":
                if last:
                    cp_out(i).start()
            elif kind == "F":
                if not last:
                    for _ in range(i):
                        if st["a"] < NC:
                            st["h"] = b_piece(sn, st["a"], st["h"], st.pop("anchor", None))
                            st["a"] += 1

        st["q", SPLIT - 1] = st["q"]
        jobs = OPTS.get("ob", "SA2.SB2.Q1.M3.M2.M1.M0.PA2.F1.O3.F1.K7.F1.PB2.F1.K6.F1.SA1.F1.SB1.F1.Q0.F1.PA1.F1.O2.F1."
                        "K5.F1.PB1.F1.K4.F1.K2.F1.SA0.SB0.K3.G0.F1.PA0.O1.F1.PB0.K1.F1.O0.F1.K0.N0").split(".")
        if last:
            jobs = OPTS.get("ol", "M3.M2.M1.M0.SA2.C7.SB2.C6.Q1.C5.C4.D4.PA2.O3.D3.PB2.SA1.SB1.Q0.PA1.O2.D2.PB1.SA0.SB0.PA0.O1.D1.PB0.O0.D0").split(".")
        for name in jobs:
            job(name)
        if not last:
            assert st["a"] == NC, st["a"]
        else:
            for i in range(SPLIT + 2):
                cp_out(i).wait()


    front_first()

    def step(s, carry):
        seg_a(s)

        @pl.when(s == 0)
        def _():
            cp_x(1).wait()
            cp_x(0).wait()
            pack_x(1)
            pack_x(0)
            cp_wo(1).wait()
            for kind in range(3):
                cp_w(kind, 1).wait()
            for kind in range(3):
                cp_b(kind, 1).start()
            cp_wo(2).start()
            for g in range(2, NG):
                for kind in range(3):
                    cp_w(kind, g).start()

        @pl.when(s == 1)
        def _():
            cp_wo(2).wait()
            for kind in range(3):
                cp_b(kind, 1).wait()

        for g in range(2, NG):
            @pl.when(s == (g - 1) * P)
            def _():
                for kind in range(3):
                    cp_w(kind, g).wait()

        @pl.when(s < NS - 1)
        def _():
            seg_b(s, False)

        @pl.when(s == NS - 1)
        def _():
            seg_b(s, True)

        return carry

    lax.fori_loop(0, NS, step, 0)


@jax.jit
def pallas_gated_mix__compressed_kv_cla__ssm_conv_h3__prompt_kernel(
    A_x: jax.Array,
    A_c_kv: jax.Array,
    A_w_q: jax.Array,
    A_w_uk: jax.Array,
    A_w_uv: jax.Array,
    A_w_o: jax.Array,
    B_q: jax.Array,
    B_k: jax.Array,
    B_v: jax.Array,
    B_shift_k: jax.Array,
    B_ssm_k: jax.Array,
    B_ssm_D: jax.Array,
    gate_w: jax.Array,
):
    del B_q
    x = A_x.reshape(S, M)
    c = A_c_kv.reshape(S, C)
    bk = B_k.reshape(S, M)
    bv = B_v.reshape(S, M)
    sh = B_shift_k.T
    fwd, inv = _dft_tables()
    fwd = jnp.asarray(fwd, dtype=bf16)
    inv = jnp.asarray(inv, dtype=bf16)

    any_spec = pl.BlockSpec(memory_space=pl.ANY)
    out = pl.pallas_call(
        _kernel,
        in_specs=[any_spec] * 14,
        out_specs=any_spec,
        out_shape=jax.ShapeDtypeStruct((S, M), bf16),
        scratch_shapes=[
            pltpu.VMEM((S, M), bf16),
            pltpu.VMEM((S, C), bf16),
            pltpu.VMEM((NG, M, G, D), bf16),
            pltpu.VMEM((NG, C, G, D), bf16),
            pltpu.VMEM((NG, C, G, D), bf16),
            pltpu.VMEM((NG + 1, M * P, D), u32),
            pltpu.VMEM((NG + 1, C * P, D), u32),
            pltpu.VMEM((NG + 1, C * P, D), u32),
            pltpu.VMEM((H, D, M), bf16),
            pltpu.VMEM((S, M), bf16),
            pltpu.VMEM((S, M), bf16),
            pltpu.VMEM((M, S), bf16),
            pltpu.VMEM((KS, M), bf16),
            pltpu.VMEM((M,), bf16),
            pltpu.VMEM((M,), bf16),
            pltpu.VMEM((2, T, T), bf16),
            pltpu.VMEM((2, T, T), bf16),
            pltpu.VMEM((NJ * 8, T), f32),
            pltpu.VMEM((2, S // 2, 2 * D), u32),
            pltpu.VMEM((TQ // 2, 2 * D), u32),
            pltpu.VMEM((TQ // 2, 2 * D), u32),
            pltpu.VMEM((TQ // 2, 2 * D), u32),
            pltpu.VMEM((6, NC, T // 2, T), f32),
            pltpu.VMEM((S, T), f32),
            pltpu.VMEM((2, TQ, D), f32),
            pltpu.VMEM((S // 2, M), u32),
            pltpu.VMEM((S // 2, C), u32),
            pltpu.VMEM((S, M), f32),
            pltpu.VMEM((S + 8, T), f32),
            pltpu.VMEM((S, T), f32),
            pltpu.VMEM((NJ, S, T), f32),
            pltpu.VMEM((S, T), f32),
            pltpu.VMEM((S, M), bf16),
            pltpu.SemaphoreType.DMA((NSEM,)),
        ],
        compiler_params=pltpu.CompilerParams(
            vmem_limit_bytes=120 * 1024 * 1024,
            shape_invariant_numerics=(OPTS.get("sin", "1") == "1"),
        ),
        name="gated_mix",
    )(x, c, A_w_q, A_w_uk, A_w_uv, A_w_o, bk, bv, B_ssm_k, sh, B_ssm_D, gate_w, fwd, inv)
    return out.reshape(1, S, M)
```

```python
import numpy as np
import jax
import jax.numpy as jnp
from jax import lax
import jax.experimental.pallas as pl
import jax.experimental.pallas.tpu as pltpu

OPTS = {}

S, M, H, D, C = 2048, 1024, 32, 128, 512
G = 8
P = G // 2
NG = H // G
NS = H // 2
T = 128
TQ = 256
NB = S // TQ
NC = S // T
NJ = M // T
KS = 4
SPLIT = 3
NEG = -1e9
OUT_CHUNKS = [tuple(int(c) for c in g) for g in OPTS.get('oc', '77_56_34_22_11_00').split('_')]
QSCALE = float(D ** -0.5 * np.log2(np.e))
bf16 = jnp.bfloat16
f32 = jnp.float32
u32 = jnp.uint32

SEM_C = 0
NCC = 4
SEM_X = SEM_C + NCC
SEM_W = SEM_X + NB
SEM_WO = SEM_W + 3 * NG
SEM_B = SEM_WO + 3
SEM_S = SEM_B + 6
SEM_O = SEM_S + 5
NSEM = SEM_O + NB


def _nt(a, b):
    return lax.dot_general(a, b, (((1,), (1,)), ((), ())), preferred_element_type=f32)


def _nn(a, b):
    return jnp.dot(a, b, preferred_element_type=f32)


def _pack(v):
    return pltpu.bitcast(v, u32)


def _unpack(v):
    return pltpu.bitcast(v, bf16)


def _unpack_pair(w32):
    lo = lax.bitcast_convert_type(w32 << 16, f32).astype(bf16)
    hi = lax.bitcast_convert_type(w32 & u32(0xFFFF0000), f32).astype(bf16)
    return jnp.concatenate([lo, hi], axis=1)


def _recip(l):
    r = pl.reciprocal(l, approx=True)
    return r * (2.0 - l * r)


def _aligned(v, n):
    return v if isinstance(v, int) else pl.multiple_of(v, n)


def _dft_tables():
    n = np.arange(T)[None, :]
    k = np.arange(T)[:, None]
    ang = 2.0 * np.pi * ((n * (2 * k + 1)) % (4 * T)) / (4 * T)
    cos, sin = np.cos(ang), np.sin(ang)
    hf = T // 2
    halves = []
    for h in range(2):
        ks = np.arange(h * hf, (h + 1) * hf)
        ks = np.concatenate([ks[0::2], ks[1::2]])
        halves.append(np.concatenate([cos[ks], -sin[ks]], axis=0))
    fwd = np.stack(halves)
    inv = np.transpose(fwd, (0, 2, 1)) / T
    return fwd.astype(np.float32), inv.astype(np.float32)


def _kernel(x_hbm, c_hbm, wq_hbm, wuk_hbm, wuv_hbm, wo_hbm, bk_hbm, bv_hbm, sk_hbm,
            sh_hbm, sd_hbm, gw_hbm, f_hbm, gi_hbm,
            o_hbm,
            x_s, c_s, wq_b, wuk_b, wuv_b, wq32, wuk32, wuv32, wo_s, bk_s, bv_s, sk_s,
            sh_s, sd_s, gw_s, f_s, gi_s, par_s,
            kv32, qa32, qb32, cx32, bst, ut, osc, x32, c32,
            acc, ybuf, bbuf, gbuf, obuf, sems):
    def cp(src, dst, sem):
        return pltpu.make_async_copy(src, dst, sems.at[sem])

    def cp_c(i):
        r = pl.ds(i * (S // NCC), S // NCC)
        return cp(c_hbm.at[r, :], c_s.at[r, :], SEM_C + i)

    def cp_x(i):
        r = pl.ds(i * TQ, TQ)
        return cp(x_hbm.at[r, :], x_s.at[r, :], SEM_X + i)

    w_hbm = (wq_hbm, wuk_hbm, wuv_hbm)
    w_b = (wq_b, wuk_b, wuv_b)
    w_32 = (wq32, wuk32, wuv32)
    w_rows = (M, C, C)

    def cp_w(kind, g):
        return cp(w_hbm[kind].at[:, pl.ds(g * G, G), :], w_b[kind].at[g], SEM_W + kind * NG + g)

    def cp_wo(part):
        r = (pl.ds(0, 2), pl.ds(2, 2), pl.ds(4, H - 4))[part]
        return cp(wo_hbm.at[r], wo_s.at[r], SEM_WO + part)

    def cp_b(kind, part):
        r = (pl.ds(0, T), pl.ds(T, M - T))[part]
        if kind == 2:
            return cp(sk_hbm.at[r, :], sk_s.at[r, :], SEM_B + 2 * kind + part)
        src, dst = ((bk_hbm, bk_s), (bv_hbm, bv_s))[kind]
        return cp(src.at[:, r], dst.at[:, r], SEM_B + 2 * kind + part)

    def cp_small(i):
        src, dst = ((sh_hbm, sh_s), (sd_hbm, sd_s), (gw_hbm, gw_s), (f_hbm, f_s), (gi_hbm, gi_s))[i]
        return cp(src, dst, SEM_S + i)

    def cp_out(k):
        lo, hi = OUT_CHUNKS[k]
        r = pl.ds(lo * TQ, (hi - lo + 1) * TQ)
        return cp(obuf.at[r, :], o_hbm.at[r, :], SEM_O + k)

    def convert(kind, g_src, g_dst, r0, nrows):
        ch = 64
        for c0 in range(0, nrows, ch):
            v = w_b[kind][g_src, pl.ds(r0 + c0, ch), :, :]
            w_32[kind][g_dst, pl.ds((r0 + c0) * P, ch * P), :] = _pack(v.reshape(ch * G, D))

    def convert_loop(kind):
        def body(c, carry):
            convert(kind, 0, 0, pl.multiple_of(c * 64, 64), 64)
            return carry

        lax.fori_loop(0, w_rows[kind] // 64, body, 0)

    def x_ready(i):
        r = pl.ds(_aligned(i * TQ, TQ), TQ)
        pltpu.make_async_copy(x_hbm.at[r, :], x_s.at[r, :], sems.at[SEM_X + i]).wait()
        xv = x_s[r, :]
        x32[pl.ds(_aligned(i * (TQ // 2), TQ // 2), TQ // 2), :] = _pack(xv)
        z = jnp.sum(xv.astype(f32) * gw_s[...].astype(f32).reshape(1, M), axis=1, keepdims=True)
        gbuf[r, :] = jnp.broadcast_to(1.0 / (1.0 + jnp.exp(-z)), (TQ, T))

    def x_ready_loop(first, count):
        def body(t, carry):
            x_ready(first - t)
            return carry

        lax.fori_loop(0, count, body, 0)

    def load_w(kind, s):
        return _unpack_pair(w_32[kind][s // P, pl.ds(s % P, w_rows[kind], stride=P), :])

    row = lax.broadcasted_iota(jnp.int32, (T, T), 0)
    col = lax.broadcasted_iota(jnp.int32, (T, T), 1)
    hf = T // 2

    def kvproj(i, wuk, wuv):
        cc = _unpack(c32[i * TQ // 2:(i + 1) * TQ // 2, :])
        r = slice(i * TQ // 2, (i + 1) * TQ // 2)
        kv32[0, r, :] = _pack(_nn(cc, wuk).astype(bf16))
        kv32[1, r, :] = _pack(_nn(cc, wuv).astype(bf16))

    def qproj(i, wq):
        return (_nn(_unpack(x32[i * TQ // 2:(i + 1) * TQ // 2, :]), wq) * QSCALE).astype(bf16)

    def scores(q, h, w):
        mask = col <= row
        k = _unpack(kv32[0, 0:w // 2, h * D:(h + 1) * D])
        s1 = _nt(q, k[0:w - T])
        s2 = _nt(q[T:], k[w - T:w])
        top_d = jnp.where(mask, s1[:T, w - 2 * T:], NEG)
        top = jnp.concatenate([s1[:T, :w - 2 * T], top_d], axis=1) if w > 2 * T else top_d
        bot = jnp.concatenate([s1[T:, :], jnp.where(mask, s2, NEG)], axis=1)
        return top, bot

    def softmax(sc):
        m = jnp.max(sc, axis=1, keepdims=True)
        p = jnp.exp2(sc - m)
        l = jnp.sum(p, axis=1, keepdims=True)
        return p.astype(bf16), l

    def pv(sc, h, w):
        top, bot = sc
        v = _unpack(kv32[1, 0:w // 2, h * D:(h + 1) * D])
        if OPTS.get("pk", "1") == "0":
            pt, lt = softmax(top)
            pb, lb = softmax(bot)
            p1 = jnp.concatenate([pt, pb[:, :w - T]], axis=0)
            o1 = _nn(p1, v[0:w - T])
            o2 = _nn(pb[:, w - T:], v[w - T:w])
            ot = o1[:T] * _recip(lt)
            ob = (o1[T:] + o2) * _recip(lb)
            return jnp.concatenate([ot, ob], axis=0).astype(bf16)
        pt = jnp.exp2(top - jnp.max(top, axis=1, keepdims=True))
        pb = jnp.exp2(bot - jnp.max(bot, axis=1, keepdims=True))
        pk = pltpu.pack_elementwise([pt, pb[:, :w - T]], packed_dtype=bf16)
        pl_ = pb[:, w - T:].astype(bf16)
        o1 = _nn(_unpack(pk), v[0:w - T])
        o2 = _nn(pl_, v[w - T:w])
        lo = pltpu.unpack_elementwise(pk, index=0, packed_dtype=bf16, unpacked_dtype=f32)
        hi = pltpu.unpack_elementwise(pk, index=1, packed_dtype=bf16, unpacked_dtype=f32)
        lt = jnp.sum(lo, axis=1, keepdims=True)
        lb = jnp.sum(jnp.concatenate([hi, pl_.astype(f32)], axis=1), axis=1, keepdims=True)
        osc[h] = o1
        ot = osc[h, pl.ds(0, T, stride=2), :] * _recip(lt)
        ob = (osc[h, pl.ds(1, T, stride=2), :] + o2) * _recip(lb)
        return jnp.concatenate([ot, ob], axis=0).astype(bf16)

    def combine(i, a):
        rows = slice(i * TQ, (i + 1) * TQ)
        g = gbuf[rows, :]
        for jj in range(NJ):
            b = bbuf[jj, rows, :]
            obuf[rows, jj * T:(jj + 1) * T] = (b + g * (a[:, jj * T:(jj + 1) * T] - b)).astype(bf16)

    def oproj(i, ctx2, wo, final=False, part=None):
        rows = slice(i * TQ, (i + 1) * TQ)
        if part is not None:
            cols = slice(part * (M // 2), (part + 1) * (M // 2))
            acc[rows, cols] = _nn(ctx2, wo[:, cols]) + acc[rows, cols]
            return
        a = _nn(ctx2, wo) + acc[rows, :]
        if final:
            combine(i, a)
        else:
            acc[rows, :] = a

    def load_wo(s):
        return wo_s[pl.ds(2 * s, 2)].reshape(2 * D, M)

    def b_piece(s, a, prev):
        j = s // 2
        jl = pl.ds(_aligned(j * T, T), T)
        rows = slice(a * T, (a + 1) * T)
        taps = par_s[pl.ds(_aligned(j * 8, 8), 8), :]
        kf = bk_s[rows, jl].astype(f32)
        ks = kf * taps[0:1, :]
        tail = prev[1] if prev is not None else jnp.zeros((8, T), f32)
        ext = jnp.concatenate([tail, kf], axis=0)
        for t in range(1, KS):
            ks = ks + pltpu.roll(ext, t, 0)[8:, :] * taps[t:t + 1, :]
        u = ks * bv_s[rows, jl].astype(f32)
        ut[rows, :] = u * taps[KS:KS + 1, :]
        fm = f_s[s % 2]
        uh = _nn(fm, u.astype(bf16))
        ur, ui = uh[0:hf], uh[hf:T]
        bst[0, a] = ur
        bst[1, a] = ui
        bst[2, a] = ur + ui
        hh = _nt(fm, sk_s[pl.ds(_aligned(j * T, T), T), rows])
        hr, hi = hh[0:hf], hh[hf:T]
        if prev is not None:
            prev_h = prev[0]
            pr, pi = prev_h[0:hf], prev_h[hf:T]
            q = hf // 2
            hr = jnp.concatenate([hr[:q] - pi[:q], hr[q:] + pi[q:]], axis=0)
            hi = jnp.concatenate([hi[:q] + pr[:q], hi[q:] - pr[q:]], axis=0)
        bst[3, a] = hr
        bst[4, a] = hi - hr
        bst[5, a] = hr + hi
        return hh, kf[T - 8:, :]

    def b_front(s):
        ph = None
        for a in range(NC):
            ph = b_piece(s, a, ph)

    def b_mac(s, c, last=False):
        k1 = k2 = k3 = None
        for a in range(c + 1):
            jj = c - a
            t1 = bst[3, jj] * bst[2, a]
            t2 = bst[0, a] * bst[4, jj]
            t3 = bst[1, a] * bst[5, jj]
            k1 = t1 if k1 is None else k1 + t1
            k2 = t2 if k2 is None else k2 + t2
            k3 = t3 if k3 is None else k3 + t3
        z = jnp.concatenate([k1 - k3, k1 + k2], axis=0).astype(bf16)
        rows = slice(c * T, (c + 1) * T)
        y = _nn(gi_s[s % 2], z)
        if last:
            y = y + ybuf[rows, :]
        else:
            y = y + jnp.where(s % 2 == 1, ybuf[rows, :], 0.0)
            ybuf[rows, :] = y
        j = s // 2
        jl = pl.ds(_aligned(j * T, T), T)
        bbuf[j, rows, :] = x_s[rows, jl].astype(f32) * (y + ut[rows, :])

    def front_first():
        cp_w(1, 0).start()
        cp_w(2, 0).start()
        for i in range(NCC):
            cp_c(i).start()
        for i in range(5):
            cp_small(i).start()
        cp_w(0, 0).start()
        cp_x(NB - 1).start()
        for kind in range(3):
            cp_b(kind, 0).start()
        for i in range(NB - 2, 1, -1):
            cp_x(i).start()
        cp_wo(0).start()
        cp_x(1).start()
        cp_x(0).start()

        def zero(i, carry):
            acc[pl.ds(pl.multiple_of(i * 64, 64), 64), :] = jnp.zeros((64, M), f32)
            return carry

        lax.fori_loop(0, S // 64, zero, 0)
        cp_w(1, 0).wait()
        convert_loop(1)
        cp_w(2, 0).wait()
        convert_loop(2)
        rc = S // NCC

        def kv_chunk(i, carry):
            r = pl.ds(pl.multiple_of(i * rc, rc), rc)
            pltpu.make_async_copy(c_hbm.at[r, :], c_s.at[r, :], sems.at[SEM_C + i]).wait()
            cc = c_s[r, :]
            rp = pl.ds(pl.multiple_of(i * (rc // 2), rc // 2), rc // 2)
            c32[rp, :] = _pack(cc)
            kv32[0, rp, :] = _pack(_nn(cc, load_w(1, 0)).astype(bf16))
            kv32[1, rp, :] = _pack(_nn(cc, load_w(2, 0)).astype(bf16))
            return carry

        lax.fori_loop(0, NCC, kv_chunk, 0)
        cp_w(0, 0).wait()
        convert_loop(0)
        for i in range(5):
            cp_small(i).wait()
        x_ready(NB - 1)
        qa32[...] = _pack(qproj(NB - 1, load_w(0, 0)))
        for kind in range(3):
            cp_b(kind, 0).wait()
        shf = sh_s[...].astype(f32)
        sdf = sd_s[...].astype(f32).reshape(1, M)
        for jj in range(NJ):
            par_s[jj * 8:jj * 8 + KS, :] = shf[:, jj * T:(jj + 1) * T]
            par_s[jj * 8 + KS:jj * 8 + KS + 1, :] = sdf[:, jj * T:(jj + 1) * T]
            par_s[jj * 8 + KS + 1:jj * 8 + 8, :] = jnp.zeros((8 - KS - 1, T), f32)
        b_front(0)
        x_ready_loop(NB - 2, NB - 3)
        cp_wo(0).wait()
        cp_wo(1).start()
        for kind in range(3):
            cp_w(kind, 1).start()

    A_DEFAULT = {7: "SA.SB.Q.M15.PA.O.M4.PB", 6: "SA.SB.Q.M14.PA.O.M5.PB", 5: "SA.SB.Q.M13.PA.O.M6.PB",
                 4: "SA.SB.Q.M12.PA.O.M7.M8.PB", 3: "SA.Q.SB.M11.PA.O.M10.M9.PB"}

    def seg_a(s):
        wq = load_w(0, s)
        wo = load_wo(s)
        qn = _unpack(qa32[...])
        prev = None
        for i in range(NB - 1, SPLIT - 1, -1):
            w = (i + 1) * TQ
            q2 = qn
            sc = [None, None]
            ctx = [None, None]
            for op in OPTS.get("A%d" % i, A_DEFAULT[i]).split("."):
                if op == "SA":
                    sc[0] = scores(q2[:, 0:D], 0, w)
                elif op == "SB":
                    sc[1] = scores(q2[:, D:2 * D], 1, w)
                elif op[0] == "M":
                    b_mac(s, int(op[1:]))
                elif op == "Q":
                    qn = qproj(i - 1, wq)
                elif op == "PA":
                    ctx[0] = pv(sc[0], 0, w)
                elif op == "PB":
                    ctx[1] = pv(sc[1], 1, w)
                elif op == "O":
                    if prev is not None:
                        oproj(i + 1, prev, wo)
                elif op in ("Oa", "Ob"):
                    if prev is not None:
                        oproj(i + 1, prev, wo, part=(0 if op == "Oa" else 1))
            prev = jnp.concatenate(ctx, axis=1)
        qb32[...] = _pack(qn)
        cx32[...] = _pack(prev)

    def seg_b(s, last):
        if not last:
            sn = s + 1
            gsrc = jnp.minimum(s // P + 1, NG - 1)
            gdst = s // P + 1
            q4 = s % P
            for kind in range(3):
                n = w_rows[kind] // P
                convert(kind, gsrc, gdst, _aligned(q4 * n, n), n)
            wuk = load_w(1, sn)
            wuv = load_w(2, sn)
        wq = load_w(0, s)
        wo = load_wo(s)
        st = {"q": _unpack(qb32[...]), "prev": _unpack(cx32[...]), "h": None, "a": 0}

        def job(name):
            kind, i = name[0], int(name[-1])
            if name[0] == "M":
                b_mac(s, i, last)
            elif name[:2] in ("SA", "SB"):
                h = 0 if name[1] == "A" else 1
                st["sc", h] = scores(st["q", i][:, h * D:(h + 1) * D], h, (i + 1) * TQ)
            elif kind == "Q":
                st["q", i] = qproj(i, wq)
            elif name[:2] in ("PA", "PB"):
                h = 0 if name[1] == "A" else 1
                st["ctx", i, h] = pv(st["sc", h], h, (i + 1) * TQ)
            elif kind == "O":
                ctx = st["prev"] if i == SPLIT else jnp.concatenate([st["ctx", i, 0], st["ctx", i, 1]], axis=1)
                oproj(i, ctx, wo, last)
            elif kind == "K":
                if not last:
                    kvproj(i, wuk, wuv)
            elif kind == "N":
                if not last:
                    qa32[...] = _pack(qproj(NB - 1, load_w(0, sn)))
            elif kind == "C":
                if last:
                    combine(i, acc[i * TQ:(i + 1) * TQ, :])
            elif kind == "D":
                if last:
                    cp_out(i).start()
            elif kind == "F":
                if not last:
                    for _ in range(i):
                        if st["a"] < NC:
                            st["h"] = b_piece(sn, st["a"], st["h"])
                            st["a"] += 1

        st["q", SPLIT - 1] = st["q"]
        jobs = OPTS.get("ob", "SA2.SB2.Q1.M3.M2.M1.M0.PA2.F1.O3.F1.K7.F1.PB2.F1.K6.F1.SA1.F1.SB1.F1.Q0.F1.PA1.F1.O2.F1."
                        "K5.F1.PB1.F1.K4.F1.K2.F1.SA0.SB0.K3.F1.PA0.O1.F1.PB0.K1.F1.O0.F1.K0.N0").split(".")
        if last:
            jobs = OPTS.get("ol", "SA2.C7.D0.SB2.C6.Q1.C5.D1.M3.M2.M1.M0.PA2.C4.O3.D2.PB2.SA1.SB1.Q0.PA1.O2.D3.PB1.SA0.SB0.PA0.O1.D4.PB0.O0.D5").split(".")
        for name in jobs:
            job(name)
        if not last:
            assert st["a"] == NC, st["a"]
        else:
            for k in range(len(OUT_CHUNKS)):
                cp_out(k).wait()


    front_first()

    def step(s, carry):
        seg_a(s)

        @pl.when(jnp.logical_and(s <= (NG - 2) * P, jnp.logical_or(s <= 1, s % P == 0)))
        def _():
            @pl.when(s == 0)
            def _():
                x_ready_loop(1, 2)
                cp_wo(1).wait()
                for kind in range(3):
                    cp_w(kind, 1).wait()
                for kind in range(3):
                    cp_b(kind, 1).start()
                cp_wo(2).start()
                for g in range(2, NG):
                    for kind in range(3):
                        cp_w(kind, g).start()

            @pl.when(s == 1)
            def _():
                cp_wo(2).wait()
                for kind in range(3):
                    cp_b(kind, 1).wait()

            for g in range(2, NG):
                @pl.when(s == (g - 1) * P)
                def _():
                    for kind in range(3):
                        cp_w(kind, g).wait()

        @pl.when(s < NS - 1)
        def _():
            seg_b(s, False)

        @pl.when(s == NS - 1)
        def _():
            seg_b(s, True)

        return carry

    lax.fori_loop(0, NS, step, 0)


@jax.jit
def pallas_gated_mix__compressed_kv_cla__ssm_conv_h3__prompt_kernel(
    A_x: jax.Array,
    A_c_kv: jax.Array,
    A_w_q: jax.Array,
    A_w_uk: jax.Array,
    A_w_uv: jax.Array,
    A_w_o: jax.Array,
    B_q: jax.Array,
    B_k: jax.Array,
    B_v: jax.Array,
    B_shift_k: jax.Array,
    B_ssm_k: jax.Array,
    B_ssm_D: jax.Array,
    gate_w: jax.Array,
):
    del B_q
    x = A_x.reshape(S, M)
    c = A_c_kv.reshape(S, C)
    bk = B_k.reshape(S, M)
    bv = B_v.reshape(S, M)
    sh = B_shift_k.T
    fwd, inv = _dft_tables()
    fwd = jnp.asarray(fwd, dtype=bf16)
    inv = jnp.asarray(inv, dtype=bf16)

    any_spec = pl.BlockSpec(memory_space=pl.ANY)
    out = pl.pallas_call(
        _kernel,
        in_specs=[any_spec] * 14,
        out_specs=any_spec,
        out_shape=jax.ShapeDtypeStruct((S, M), bf16),
        scratch_shapes=[
            pltpu.VMEM((S, M), bf16),
            pltpu.VMEM((S, C), bf16),
            pltpu.VMEM((NG, M, G, D), bf16),
            pltpu.VMEM((NG, C, G, D), bf16),
            pltpu.VMEM((NG, C, G, D), bf16),
            pltpu.VMEM((NG + 1, M * P, D), u32),
            pltpu.VMEM((NG + 1, C * P, D), u32),
            pltpu.VMEM((NG + 1, C * P, D), u32),
            pltpu.VMEM((H, D, M), bf16),
            pltpu.VMEM((S, M), bf16),
            pltpu.VMEM((S, M), bf16),
            pltpu.VMEM((M, S), bf16),
            pltpu.VMEM((KS, M), bf16),
            pltpu.VMEM((M,), bf16),
            pltpu.VMEM((M,), bf16),
            pltpu.VMEM((2, T, T), bf16),
            pltpu.VMEM((2, T, T), bf16),
            pltpu.VMEM((NJ * 8, T), f32),
            pltpu.VMEM((2, S // 2, 2 * D), u32),
            pltpu.VMEM((TQ // 2, 2 * D), u32),
            pltpu.VMEM((TQ // 2, 2 * D), u32),
            pltpu.VMEM((TQ // 2, 2 * D), u32),
            pltpu.VMEM((6, NC, T // 2, T), f32),
            pltpu.VMEM((S, T), f32),
            pltpu.VMEM((2, TQ, D), f32),
            pltpu.VMEM((S // 2, M), u32),
            pltpu.VMEM((S // 2, C), u32),
            pltpu.VMEM((S, M), f32),
            pltpu.VMEM((S, T), f32),
            pltpu.VMEM((NJ, S, T), f32),
            pltpu.VMEM((S, T), f32),
            pltpu.VMEM((S, M), bf16),
            pltpu.SemaphoreType.DMA((NSEM,)),
        ],
        compiler_params=pltpu.CompilerParams(
            vmem_limit_bytes=120 * 1024 * 1024,
            shape_invariant_numerics=(OPTS.get("sin", "1") == "1"),
        ),
        name="gated_mix",
    )(x, c, A_w_q, A_w_uk, A_w_uv, A_w_o, bk, bv, B_ssm_k, sh, B_ssm_D, gate_w, fwd, inv)
    return out.reshape(1, S, M)
```

```python
import numpy as np
import jax
import jax.numpy as jnp
from jax import lax
import jax.experimental.pallas as pl
import jax.experimental.pallas.tpu as pltpu

OPTS = {}

S, M, H, D, C = 2048, 1024, 32, 128, 512
G = 8
P = G // 2
NG = H // G
NS = H // 2
T = 128
TQ = 256
NB = S // TQ
NC = S // T
NJ = M // T
KS = 4
SPLIT = 3
NEG = -1e9
DEFER = OPTS.get('df', '1') == '1'
OUT_CHUNKS = [tuple(int(c) for c in g) for g in OPTS.get('oc', '77_56_34_22_11_00').split('_')]
QSCALE = float(D ** -0.5 * np.log2(np.e))
bf16 = jnp.bfloat16
f32 = jnp.float32
u32 = jnp.uint32

SEM_C = 0
NCC = 4
SEM_X = SEM_C + NCC
SEM_W = SEM_X + NB
SEM_WO = SEM_W + 3 * NG
SEM_B = SEM_WO + 3
SEM_S = SEM_B + 6
SEM_O = SEM_S + 5
NSEM = SEM_O + NB


def _nt(a, b):
    return lax.dot_general(a, b, (((1,), (1,)), ((), ())), preferred_element_type=f32)


def _nn(a, b):
    return jnp.dot(a, b, preferred_element_type=f32)


def _pack(v):
    return pltpu.bitcast(v, u32)


def _unpack(v):
    return pltpu.bitcast(v, bf16)


def _unpack_pair(w32):
    lo = lax.bitcast_convert_type(w32 << 16, f32).astype(bf16)
    hi = lax.bitcast_convert_type(w32 & u32(0xFFFF0000), f32).astype(bf16)
    return jnp.concatenate([lo, hi], axis=1)


def _recip(l):
    r = pl.reciprocal(l, approx=True)
    return r * (2.0 - l * r)


def _aligned(v, n):
    return v if isinstance(v, int) else pl.multiple_of(v, n)


def _dft_tables():
    n = np.arange(T)[None, :]
    k = np.arange(T)[:, None]
    ang = 2.0 * np.pi * ((n * (2 * k + 1)) % (4 * T)) / (4 * T)
    cos, sin = np.cos(ang), np.sin(ang)
    hf = T // 2
    halves = []
    for h in range(2):
        ks = np.arange(h * hf, (h + 1) * hf)
        ks = np.concatenate([ks[0::2], ks[1::2]])
        halves.append(np.concatenate([cos[ks], -sin[ks]], axis=0))
    fwd = np.stack(halves)
    inv = np.transpose(fwd, (0, 2, 1)) / T
    return fwd.astype(np.float32), inv.astype(np.float32)


def _kernel(x_hbm, c_hbm, wq_hbm, wuk_hbm, wuv_hbm, wo_hbm, bk_hbm, bv_hbm, sk_hbm,
            sh_hbm, sd_hbm, gw_hbm, f_hbm, gi_hbm,
            o_hbm,
            x_s, c_s, wq_b, wuk_b, wuv_b, wq32, wuk32, wuv32, wo_s, bk_s, bv_s, sk_s,
            sh_s, sd_s, gw_s, f_s, gi_s, par_s,
            kv32, qa32, qb32, cx32, bst, ut, osc, x32, c32, dsc,
            acc, ybuf, bbuf, gbuf, obuf, sems):
    def cp(src, dst, sem):
        return pltpu.make_async_copy(src, dst, sems.at[sem])

    def cp_c(i):
        r = pl.ds(i * (S // NCC), S // NCC)
        return cp(c_hbm.at[r, :], c_s.at[r, :], SEM_C + i)

    def cp_x(i):
        r = pl.ds(i * TQ, TQ)
        return cp(x_hbm.at[r, :], x_s.at[r, :], SEM_X + i)

    w_hbm = (wq_hbm, wuk_hbm, wuv_hbm)
    w_b = (wq_b, wuk_b, wuv_b)
    w_32 = (wq32, wuk32, wuv32)
    w_rows = (M, C, C)

    def cp_w(kind, g):
        return cp(w_hbm[kind].at[:, pl.ds(g * G, G), :], w_b[kind].at[g], SEM_W + kind * NG + g)

    def cp_wo(part):
        r = (pl.ds(0, 2), pl.ds(2, 2), pl.ds(4, H - 4))[part]
        return cp(wo_hbm.at[r], wo_s.at[r], SEM_WO + part)

    def cp_b(kind, part):
        r = (pl.ds(0, T), pl.ds(T, M - T))[part]
        if kind == 2:
            return cp(sk_hbm.at[r, :], sk_s.at[r, :], SEM_B + 2 * kind + part)
        src, dst = ((bk_hbm, bk_s), (bv_hbm, bv_s))[kind]
        return cp(src.at[:, r], dst.at[:, r], SEM_B + 2 * kind + part)

    def cp_small(i):
        src, dst = ((sh_hbm, sh_s), (sd_hbm, sd_s), (gw_hbm, gw_s), (f_hbm, f_s), (gi_hbm, gi_s))[i]
        return cp(src, dst, SEM_S + i)

    def cp_out(k):
        lo, hi = OUT_CHUNKS[k]
        r = pl.ds(lo * TQ, (hi - lo + 1) * TQ)
        return cp(obuf.at[r, :], o_hbm.at[r, :], SEM_O + k)

    def convert(kind, g_src, g_dst, r0, nrows):
        ch = 64
        for c0 in range(0, nrows, ch):
            v = w_b[kind][g_src, pl.ds(r0 + c0, ch), :, :]
            w_32[kind][g_dst, pl.ds((r0 + c0) * P, ch * P), :] = _pack(v.reshape(ch * G, D))

    def convert_loop(kind):
        def body(c, carry):
            convert(kind, 0, 0, pl.multiple_of(c * 64, 64), 64)
            return carry

        lax.fori_loop(0, w_rows[kind] // 64, body, 0)

    def x_ready(i):
        r = pl.ds(_aligned(i * TQ, TQ), TQ)
        pltpu.make_async_copy(x_hbm.at[r, :], x_s.at[r, :], sems.at[SEM_X + i]).wait()
        xv = x_s[r, :]
        x32[pl.ds(_aligned(i * (TQ // 2), TQ // 2), TQ // 2), :] = _pack(xv)
        z = jnp.sum(xv.astype(f32) * gw_s[...].astype(f32).reshape(1, M), axis=1, keepdims=True)
        gbuf[r, :] = jnp.broadcast_to(1.0 / (1.0 + jnp.exp(-z)), (TQ, T))

    def x_ready_loop(first, count):
        def body(t, carry):
            x_ready(first - t)
            return carry

        lax.fori_loop(0, count, body, 0)

    def load_w(kind, s):
        return _unpack_pair(w_32[kind][s // P, pl.ds(s % P, w_rows[kind], stride=P), :])

    row = lax.broadcasted_iota(jnp.int32, (T, T), 0)
    col = lax.broadcasted_iota(jnp.int32, (T, T), 1)
    hf = T // 2

    def kvproj(i, wuk, wuv):
        cc = _unpack(c32[i * TQ // 2:(i + 1) * TQ // 2, :])
        r = slice(i * TQ // 2, (i + 1) * TQ // 2)
        kv32[0, r, :] = _pack(_nn(cc, wuk).astype(bf16))
        kv32[1, r, :] = _pack(_nn(cc, wuv).astype(bf16))

    def qproj(i, wq):
        return (_nn(_unpack(x32[i * TQ // 2:(i + 1) * TQ // 2, :]), wq) * QSCALE).astype(bf16)

    def scores(q, h, w):
        mask = col <= row
        k = _unpack(kv32[0, 0:w // 2, h * D:(h + 1) * D])
        s1 = _nt(q, k[0:w - T])
        s2 = _nt(q[T:], k[w - T:w])
        top_d = jnp.where(mask, s1[:T, w - 2 * T:], NEG)
        top = jnp.concatenate([s1[:T, :w - 2 * T], top_d], axis=1) if w > 2 * T else top_d
        bot = jnp.concatenate([s1[T:, :], jnp.where(mask, s2, NEG)], axis=1)
        return top, bot

    def softmax(sc):
        m = jnp.max(sc, axis=1, keepdims=True)
        p = jnp.exp2(sc - m)
        l = jnp.sum(p, axis=1, keepdims=True)
        return p.astype(bf16), l

    def pv(sc, h, w, defer=False):
        top, bot = sc
        v = _unpack(kv32[1, 0:w // 2, h * D:(h + 1) * D])
        pt = jnp.exp2(top - jnp.max(top, axis=1, keepdims=True))
        pb = jnp.exp2(bot - jnp.max(bot, axis=1, keepdims=True))
        ut_ = lax.bitcast_convert_type(pt, u32)
        ub_ = lax.bitcast_convert_type(pb[:, :w - T], u32)
        if OPTS.get("rnd", "trunc") == "trunc":
            pk = (ut_ >> 16) | (ub_ & u32(0xFFFF0000))
        elif OPTS["rnd"] == "rhu":
            pk = ((ut_ + u32(0x8000)) >> 16) | ((ub_ + u32(0x8000)) & u32(0xFFFF0000))
        else:
            pk = pltpu.pack_elementwise([pt, pb[:, :w - T]], packed_dtype=bf16)
        pl_ = pb[:, w - T:].astype(bf16)
        o1 = _nn(_unpack(pk), v[0:w - T])
        o2 = _nn(pl_, v[w - T:w])
        lo = lax.bitcast_convert_type(pk << 16, f32)
        hi = lax.bitcast_convert_type(pk & u32(0xFFFF0000), f32)
        lt = jnp.sum(lo, axis=1, keepdims=True)
        lb = jnp.sum(jnp.concatenate([hi, pl_.astype(f32)], axis=1), axis=1, keepdims=True)
        osc[h] = o1
        if defer:
            dsc[0] = o2
            dsc[1] = jnp.broadcast_to(lt, (T, D))
            dsc[2] = jnp.broadcast_to(lb, (T, D))
            return None
        return pv_finish(h, o2, lt, lb)

    def pv_finish(h, o2, lt, lb):
        ot = osc[h, pl.ds(0, T, stride=2), :] * _recip(lt)
        ob = (osc[h, pl.ds(1, T, stride=2), :] + o2) * _recip(lb)
        return jnp.concatenate([ot, ob], axis=0).astype(bf16)

    def combine(i, a):
        rows = slice(i * TQ, (i + 1) * TQ)
        g = gbuf[rows, :]
        for jj in range(NJ):
            b = bbuf[jj, rows, :]
            obuf[rows, jj * T:(jj + 1) * T] = (b + g * (a[:, jj * T:(jj + 1) * T] - b)).astype(bf16)

    def oproj(i, ctx2, wo, final=False, part=None):
        rows = slice(i * TQ, (i + 1) * TQ)
        if part is not None:
            cols = slice(part * (M // 2), (part + 1) * (M // 2))
            acc[rows, cols] = _nn(ctx2, wo[:, cols]) + acc[rows, cols]
            return
        a = _nn(ctx2, wo) + acc[rows, :]
        if final:
            combine(i, a)
        else:
            acc[rows, :] = a

    def load_wo(s):
        return wo_s[pl.ds(2 * s, 2)].reshape(2 * D, M)

    def b_piece(s, a, prev):
        j = s // 2
        jl = pl.ds(_aligned(j * T, T), T)
        rows = slice(a * T, (a + 1) * T)
        taps = par_s[pl.ds(_aligned(j * 8, 8), 8), :]
        kf = bk_s[rows, jl].astype(f32)
        ks = kf * taps[0:1, :]
        tail = prev[1] if prev is not None else jnp.zeros((8, T), f32)
        ext = jnp.concatenate([tail, kf], axis=0)
        for t in range(1, KS):
            ks = ks + pltpu.roll(ext, t, 0)[8:, :] * taps[t:t + 1, :]
        u = ks * bv_s[rows, jl].astype(f32)
        ut[rows, :] = u * taps[KS:KS + 1, :]
        fm = f_s[s % 2]
        uh = _nn(fm, u.astype(bf16))
        ur, ui = uh[0:hf], uh[hf:T]
        bst[0, a] = ur
        bst[1, a] = ui
        bst[2, a] = ur + ui
        hh = _nt(fm, sk_s[pl.ds(_aligned(j * T, T), T), rows])
        hr, hi = hh[0:hf], hh[hf:T]
        if prev is not None:
            prev_h = prev[0]
            pr, pi = prev_h[0:hf], prev_h[hf:T]
            q = hf // 2
            hr = jnp.concatenate([hr[:q] - pi[:q], hr[q:] + pi[q:]], axis=0)
            hi = jnp.concatenate([hi[:q] + pr[:q], hi[q:] - pr[q:]], axis=0)
        bst[3, a] = hr
        bst[4, a] = hi - hr
        bst[5, a] = hr + hi
        return hh, kf[T - 8:, :]

    def b_front(s):
        ph = None
        for a in range(NC):
            ph = b_piece(s, a, ph)

    def b_mac(s, c, last=False):
        k1 = k2 = k3 = None
        for a in range(c + 1):
            jj = c - a
            t1 = bst[3, jj] * bst[2, a]
            t2 = bst[0, a] * bst[4, jj]
            t3 = bst[1, a] * bst[5, jj]
            k1 = t1 if k1 is None else k1 + t1
            k2 = t2 if k2 is None else k2 + t2
            k3 = t3 if k3 is None else k3 + t3
        z = jnp.concatenate([k1 - k3, k1 + k2], axis=0).astype(bf16)
        rows = slice(c * T, (c + 1) * T)
        y = _nn(gi_s[s % 2], z)
        if last:
            y = y + ybuf[rows, :]
        else:
            y = y + jnp.where(s % 2 == 1, ybuf[rows, :], 0.0)
            ybuf[rows, :] = y
        j = s // 2
        jl = pl.ds(_aligned(j * T, T), T)
        bbuf[j, rows, :] = x_s[rows, jl].astype(f32) * (y + ut[rows, :])

    def front_first():
        cp_w(1, 0).start()
        cp_w(2, 0).start()
        for i in range(NCC):
            cp_c(i).start()
        for i in range(5):
            cp_small(i).start()
        cp_w(0, 0).start()
        cp_x(NB - 1).start()
        for kind in range(3):
            cp_b(kind, 0).start()
        for i in range(NB - 2, 1, -1):
            cp_x(i).start()
        cp_wo(0).start()
        cp_x(1).start()
        cp_x(0).start()

        def zero(i, carry):
            acc[pl.ds(pl.multiple_of(i * 64, 64), 64), :] = jnp.zeros((64, M), f32)
            return carry

        lax.fori_loop(0, S // 64, zero, 0)
        cp_w(1, 0).wait()
        convert_loop(1)
        cp_w(2, 0).wait()
        convert_loop(2)
        rc = S // NCC

        def kv_chunk(i, carry):
            r = pl.ds(pl.multiple_of(i * rc, rc), rc)
            pltpu.make_async_copy(c_hbm.at[r, :], c_s.at[r, :], sems.at[SEM_C + i]).wait()
            cc = c_s[r, :]
            rp = pl.ds(pl.multiple_of(i * (rc // 2), rc // 2), rc // 2)
            c32[rp, :] = _pack(cc)
            kv32[0, rp, :] = _pack(_nn(cc, load_w(1, 0)).astype(bf16))
            kv32[1, rp, :] = _pack(_nn(cc, load_w(2, 0)).astype(bf16))
            return carry

        lax.fori_loop(0, NCC, kv_chunk, 0)
        cp_w(0, 0).wait()
        convert_loop(0)
        for i in range(5):
            cp_small(i).wait()
        x_ready(NB - 1)
        qa32[...] = _pack(qproj(NB - 1, load_w(0, 0)))
        for kind in range(3):
            cp_b(kind, 0).wait()
        shf = sh_s[...].astype(f32)
        sdf = sd_s[...].astype(f32).reshape(1, M)
        for jj in range(NJ):
            par_s[jj * 8:jj * 8 + KS, :] = shf[:, jj * T:(jj + 1) * T]
            par_s[jj * 8 + KS:jj * 8 + KS + 1, :] = sdf[:, jj * T:(jj + 1) * T]
            par_s[jj * 8 + KS + 1:jj * 8 + 8, :] = jnp.zeros((8 - KS - 1, T), f32)
        b_front(0)
        x_ready_loop(NB - 2, NB - 3)
        cp_wo(0).wait()
        cp_wo(1).start()
        for kind in range(3):
            cp_w(kind, 1).start()

    A_DEFAULT = {7: "SA.SB.Q.M15.PA.O.M4.PB", 6: "SA.SB.Q.M14.PA.O.M5.PB", 5: "SA.SB.Q.M13.PA.O.M6.PB",
                 4: "SA.SB.Q.M12.PA.O.M7.M8.PB", 3: "SA.Q.SB.M11.PA.O.M10.M9.PB"}

    def seg_a(s):
        wq = load_w(0, s)
        wo = load_wo(s)
        qn = _unpack(qa32[...])
        prev = None
        for i in range(NB - 1, SPLIT - 1, -1):
            w = (i + 1) * TQ
            q2 = qn
            sc = [None, None]
            ctx = [None, None]
            for op in OPTS.get("A%d" % i, A_DEFAULT[i]).split("."):
                if op == "SA":
                    sc[0] = scores(q2[:, 0:D], 0, w)
                elif op == "SB":
                    sc[1] = scores(q2[:, D:2 * D], 1, w)
                elif op[0] == "M":
                    b_mac(s, int(op[1:]))
                elif op == "Q":
                    qn = qproj(i - 1, wq)
                elif op == "PA":
                    ctx[0] = pv(sc[0], 0, w)
                elif op == "PB":
                    ctx[1] = pv(sc[1], 1, w, defer=(DEFER and i == SPLIT))
                    if ctx[1] is None:
                        ctx[1] = ctx[0]
                elif op == "O":
                    if prev is not None:
                        oproj(i + 1, prev, wo)
                elif op in ("Oa", "Ob"):
                    if prev is not None:
                        oproj(i + 1, prev, wo, part=(0 if op == "Oa" else 1))
            prev = jnp.concatenate(ctx, axis=1)
        qb32[...] = _pack(qn)
        cx32[...] = _pack(prev)

    def seg_b(s, last):
        if not last:
            sn = s + 1
            gsrc = jnp.minimum(s // P + 1, NG - 1)
            gdst = s // P + 1
            q4 = s % P
            for kind in range(3):
                n = w_rows[kind] // P
                convert(kind, gsrc, gdst, _aligned(q4 * n, n), n)
            wuk = load_w(1, sn)
            wuv = load_w(2, sn)
        wq = load_w(0, s)
        wo = load_wo(s)
        st = {"q": _unpack(qb32[...]), "prev": _unpack(cx32[...]), "h": None, "a": 0}
        if DEFER:
            st["prev"] = jnp.concatenate([st["prev"][:, 0:D], pv_finish(1, dsc[0], dsc[1], dsc[2])], axis=1)

        def job(name):
            kind, i = name[0], int(name[-1])
            if name[0] == "M":
                b_mac(s, i, last)
            elif name[:2] in ("SA", "SB"):
                h = 0 if name[1] == "A" else 1
                st["sc", h] = scores(st["q", i][:, h * D:(h + 1) * D], h, (i + 1) * TQ)
            elif kind == "Q":
                st["q", i] = qproj(i, wq)
            elif name[:2] in ("PA", "PB"):
                h = 0 if name[1] == "A" else 1
                st["ctx", i, h] = pv(st["sc", h], h, (i + 1) * TQ)
            elif kind == "O":
                ctx = st["prev"] if i == SPLIT else jnp.concatenate([st["ctx", i, 0], st["ctx", i, 1]], axis=1)
                oproj(i, ctx, wo, last)
            elif kind == "K":
                if not last:
                    kvproj(i, wuk, wuv)
            elif kind == "N":
                if not last:
                    qa32[...] = _pack(qproj(NB - 1, load_w(0, sn)))
            elif kind == "C":
                if last:
                    combine(i, acc[i * TQ:(i + 1) * TQ, :])
            elif kind == "D":
                if last:
                    cp_out(i).start()
            elif kind == "F":
                if not last:
                    for _ in range(i):
                        if st["a"] < NC:
                            st["h"] = b_piece(sn, st["a"], st["h"])
                            st["a"] += 1

        st["q", SPLIT - 1] = st["q"]
        jobs = OPTS.get("ob", "SA2.SB2.Q1.M3.M2.M1.M0.PA2.F1.O3.F1.K7.F1.PB2.F1.K6.F1.SA1.F1.SB1.F1.Q0.F1.PA1.F1.O2.F1."
                        "K5.F1.PB1.F1.K4.F1.K2.F1.SA0.SB0.K3.F1.PA0.O1.F1.PB0.K1.F1.O0.F1.K0.N0").split(".")
        if last:
            jobs = OPTS.get("ol", "SA2.C7.D0.SB2.C6.Q1.C5.D1.M3.M2.M1.M0.PA2.C4.O3.D2.PB2.SA1.SB1.Q0.PA1.O2.D3.PB1.SA0.SB0.PA0.O1.D4.PB0.O0.D5").split(".")
        for name in jobs:
            job(name)
        if not last:
            assert st["a"] == NC, st["a"]
        else:
            for k in range(len(OUT_CHUNKS)):
                cp_out(k).wait()


    front_first()

    def step(s, carry):
        seg_a(s)

        @pl.when(jnp.logical_and(s <= (NG - 2) * P, jnp.logical_or(s <= 1, s % P == 0)))
        def _():
            @pl.when(s == 0)
            def _():
                x_ready_loop(1, 2)
                cp_wo(1).wait()
                for kind in range(3):
                    cp_w(kind, 1).wait()
                for kind in range(3):
                    cp_b(kind, 1).start()
                cp_wo(2).start()
                for g in range(2, NG):
                    for kind in range(3):
                        cp_w(kind, g).start()

            @pl.when(s == 1)
            def _():
                cp_wo(2).wait()
                for kind in range(3):
                    cp_b(kind, 1).wait()

            for g in range(2, NG):
                @pl.when(s == (g - 1) * P)
                def _():
                    for kind in range(3):
                        cp_w(kind, g).wait()

        @pl.when(s < NS - 1)
        def _():
            seg_b(s, False)

        @pl.when(s == NS - 1)
        def _():
            seg_b(s, True)

        return carry

    lax.fori_loop(0, NS, step, 0)


@jax.jit
def pallas_gated_mix__compressed_kv_cla__ssm_conv_h3__prompt_kernel(
    A_x: jax.Array,
    A_c_kv: jax.Array,
    A_w_q: jax.Array,
    A_w_uk: jax.Array,
    A_w_uv: jax.Array,
    A_w_o: jax.Array,
    B_q: jax.Array,
    B_k: jax.Array,
    B_v: jax.Array,
    B_shift_k: jax.Array,
    B_ssm_k: jax.Array,
    B_ssm_D: jax.Array,
    gate_w: jax.Array,
):
    del B_q
    x = A_x.reshape(S, M)
    c = A_c_kv.reshape(S, C)
    bk = B_k.reshape(S, M)
    bv = B_v.reshape(S, M)
    sh = B_shift_k.T
    fwd, inv = _dft_tables()
    fwd = jnp.asarray(fwd, dtype=bf16)
    inv = jnp.asarray(inv, dtype=bf16)

    any_spec = pl.BlockSpec(memory_space=pl.ANY)
    out = pl.pallas_call(
        _kernel,
        in_specs=[any_spec] * 14,
        out_specs=any_spec,
        out_shape=jax.ShapeDtypeStruct((S, M), bf16),
        scratch_shapes=[
            pltpu.VMEM((S, M), bf16),
            pltpu.VMEM((S, C), bf16),
            pltpu.VMEM((NG, M, G, D), bf16),
            pltpu.VMEM((NG, C, G, D), bf16),
            pltpu.VMEM((NG, C, G, D), bf16),
            pltpu.VMEM((NG + 1, M * P, D), u32),
            pltpu.VMEM((NG + 1, C * P, D), u32),
            pltpu.VMEM((NG + 1, C * P, D), u32),
            pltpu.VMEM((H, D, M), bf16),
            pltpu.VMEM((S, M), bf16),
            pltpu.VMEM((S, M), bf16),
            pltpu.VMEM((M, S), bf16),
            pltpu.VMEM((KS, M), bf16),
            pltpu.VMEM((M,), bf16),
            pltpu.VMEM((M,), bf16),
            pltpu.VMEM((2, T, T), bf16),
            pltpu.VMEM((2, T, T), bf16),
            pltpu.VMEM((NJ * 8, T), f32),
            pltpu.VMEM((2, S // 2, 2 * D), u32),
            pltpu.VMEM((TQ // 2, 2 * D), u32),
            pltpu.VMEM((TQ // 2, 2 * D), u32),
            pltpu.VMEM((TQ // 2, 2 * D), u32),
            pltpu.VMEM((6, NC, T // 2, T), f32),
            pltpu.VMEM((S, T), f32),
            pltpu.VMEM((2, TQ, D), f32),
            pltpu.VMEM((S // 2, M), u32),
            pltpu.VMEM((S // 2, C), u32),
            pltpu.VMEM((3, T, D), f32),
            pltpu.VMEM((S, M), f32),
            pltpu.VMEM((S, T), f32),
            pltpu.VMEM((NJ, S, T), f32),
            pltpu.VMEM((S, T), f32),
            pltpu.VMEM((S, M), bf16),
            pltpu.SemaphoreType.DMA((NSEM,)),
        ],
        compiler_params=pltpu.CompilerParams(
            vmem_limit_bytes=120 * 1024 * 1024,
            shape_invariant_numerics=(OPTS.get("sin", "1") == "1"),
        ),
        name="gated_mix",
    )(x, c, A_w_q, A_w_uk, A_w_uv, A_w_o, bk, bv, B_ssm_k, sh, B_ssm_D, gate_w, fwd, inv)
    return out.reshape(1, S, M)
```

```python
import numpy as np
import jax
import jax.numpy as jnp
from jax import lax
import jax.experimental.pallas as pl
import jax.experimental.pallas.tpu as pltpu

S, M, H, D, C = 2048, 1024, 32, 128, 512
G = 8
P = G // 2
NG = H // G
NS = H // 2
T = 128
TQ = 256
NB = S // TQ
NC = S // T
NJ = M // T
KS = 4
SPLIT = 3
NEG = -1e9
OUT_CHUNKS = [(7, 7), (5, 6), (3, 4), (2, 2), (1, 1), (0, 0)]
QSCALE = float(D ** -0.5 * np.log2(np.e))
bf16 = jnp.bfloat16
f32 = jnp.float32
u32 = jnp.uint32

ORDER_A = {7: "SA.SB.Q.M15.PA.O.M4.PB", 6: "SA.SB.Q.M14.PA.O.M5.PB", 5: "SA.SB.Q.M13.PA.O.M6.PB",
           4: "SA.SB.Q.M12.PA.O.M7.M8.PB", 3: "SA.Q.SB.M11.PA.O.M10.M9.PB"}
ORDER_B = ("SA2.SB2.Q1.M3.M2.M1.M0.PA2.F1.O3.F1.K7.F1.PB2.F1.K6.F1.SA1.F1.SB1.F1.Q0.F1.PA1.F1.O2.F1."
           "K5.F1.PB1.F1.K4.F1.K2.F1.SA0.SB0.K3.F1.PA0.O1.F1.PB0.K1.F1.O0.F1.K0.N0")
ORDER_LAST = ("SA2.C7.D0.SB2.C6.Q1.C5.D1.M3.M2.M1.M0.PA2.C4.O3.D2.PB2.SA1.SB1.Q0.PA1.O2.D3."
              "PB1.SA0.SB0.PA0.O1.D4.PB0.O0.D5")

NCC = 4
SEM_C = 0
SEM_X = SEM_C + NCC
SEM_W = SEM_X + NB
SEM_WO = SEM_W + 3 * NG
SEM_B = SEM_WO + 3
SEM_S = SEM_B + 6
SEM_O = SEM_S + 5
NSEM = SEM_O + len(OUT_CHUNKS)


def _nt(a, b):
    return lax.dot_general(a, b, (((1,), (1,)), ((), ())), preferred_element_type=f32)


def _nn(a, b):
    return jnp.dot(a, b, preferred_element_type=f32)


def _pack(v):
    return pltpu.bitcast(v, u32)


def _unpack(v):
    return pltpu.bitcast(v, bf16)


def _unpack_pair(w32):
    lo = lax.bitcast_convert_type(w32 << 16, f32).astype(bf16)
    hi = lax.bitcast_convert_type(w32 & u32(0xFFFF0000), f32).astype(bf16)
    return jnp.concatenate([lo, hi], axis=1)


def _recip(l):
    r = pl.reciprocal(l, approx=True)
    return r * (2.0 - l * r)


def _aligned(v, n):
    return v if isinstance(v, int) else pl.multiple_of(v, n)


def _dft_tables():
    n = np.arange(T)[None, :]
    k = np.arange(T)[:, None]
    ang = 2.0 * np.pi * ((n * (2 * k + 1)) % (4 * T)) / (4 * T)
    cos, sin = np.cos(ang), np.sin(ang)
    hf = T // 2
    halves = []
    for h in range(2):
        ks = np.arange(h * hf, (h + 1) * hf)
        ks = np.concatenate([ks[0::2], ks[1::2]])
        halves.append(np.concatenate([cos[ks], -sin[ks]], axis=0))
    fwd = np.stack(halves)
    inv = np.transpose(fwd, (0, 2, 1)) / T
    return fwd.astype(np.float32), inv.astype(np.float32)


def _kernel(x_hbm, c_hbm, wq_hbm, wuk_hbm, wuv_hbm, wo_hbm, bk_hbm, bv_hbm, sk_hbm,
            sh_hbm, sd_hbm, gw_hbm, f_hbm, gi_hbm,
            o_hbm,
            x_s, c_s, wq_b, wuk_b, wuv_b, wq32, wuk32, wuv32, wo_s, bk_s, bv_s, sk_s,
            sh_s, sd_s, gw_s, f_s, gi_s, par_s,
            kv32, qa32, qb32, cx32, bst, ut, osc, x32, c32, dsc,
            acc, ybuf, bbuf, gbuf, obuf, sems):
    def cp(src, dst, sem):
        return pltpu.make_async_copy(src, dst, sems.at[sem])

    def cp_c(i):
        r = pl.ds(i * (S // NCC), S // NCC)
        return cp(c_hbm.at[r, :], c_s.at[r, :], SEM_C + i)

    def cp_x(i):
        r = pl.ds(i * TQ, TQ)
        return cp(x_hbm.at[r, :], x_s.at[r, :], SEM_X + i)

    w_hbm = (wq_hbm, wuk_hbm, wuv_hbm)
    w_b = (wq_b, wuk_b, wuv_b)
    w_32 = (wq32, wuk32, wuv32)
    w_rows = (M, C, C)

    def cp_w(kind, g):
        return cp(w_hbm[kind].at[:, pl.ds(g * G, G), :], w_b[kind].at[g], SEM_W + kind * NG + g)

    def cp_wo(part):
        r = (pl.ds(0, 2), pl.ds(2, 2), pl.ds(4, H - 4))[part]
        return cp(wo_hbm.at[r], wo_s.at[r], SEM_WO + part)

    def cp_b(kind, part):
        r = (pl.ds(0, T), pl.ds(T, M - T))[part]
        if kind == 2:
            return cp(sk_hbm.at[r, :], sk_s.at[r, :], SEM_B + 2 * kind + part)
        src, dst = ((bk_hbm, bk_s), (bv_hbm, bv_s))[kind]
        return cp(src.at[:, r], dst.at[:, r], SEM_B + 2 * kind + part)

    def cp_small(i):
        src, dst = ((sh_hbm, sh_s), (sd_hbm, sd_s), (gw_hbm, gw_s), (f_hbm, f_s), (gi_hbm, gi_s))[i]
        return cp(src, dst, SEM_S + i)

    def cp_out(k):
        lo, hi = OUT_CHUNKS[k]
        r = pl.ds(lo * TQ, (hi - lo + 1) * TQ)
        return cp(obuf.at[r, :], o_hbm.at[r, :], SEM_O + k)

    def convert(kind, g_src, g_dst, r0, nrows):
        ch = 64
        for c0 in range(0, nrows, ch):
            v = w_b[kind][g_src, pl.ds(r0 + c0, ch), :, :]
            w_32[kind][g_dst, pl.ds((r0 + c0) * P, ch * P), :] = _pack(v.reshape(ch * G, D))

    def convert_loop(kind):
        def body(c, carry):
            convert(kind, 0, 0, pl.multiple_of(c * 64, 64), 64)
            return carry

        lax.fori_loop(0, w_rows[kind] // 64, body, 0)

    def x_ready(i):
        r = pl.ds(_aligned(i * TQ, TQ), TQ)
        pltpu.make_async_copy(x_hbm.at[r, :], x_s.at[r, :], sems.at[SEM_X + i]).wait()
        xv = x_s[r, :]
        x32[pl.ds(_aligned(i * (TQ // 2), TQ // 2), TQ // 2), :] = _pack(xv)
        z = jnp.sum(xv.astype(f32) * gw_s[...].astype(f32).reshape(1, M), axis=1, keepdims=True)
        gbuf[r, :] = jnp.broadcast_to(1.0 / (1.0 + jnp.exp(-z)), (TQ, T))

    def x_ready_loop(first, count):
        def body(t, carry):
            x_ready(first - t)
            return carry

        lax.fori_loop(0, count, body, 0)

    def load_w(kind, s):
        return _unpack_pair(w_32[kind][s // P, pl.ds(s % P, w_rows[kind], stride=P), :])

    row = lax.broadcasted_iota(jnp.int32, (T, T), 0)
    col = lax.broadcasted_iota(jnp.int32, (T, T), 1)
    hf = T // 2

    def kvproj(i, wuk, wuv):
        cc = _unpack(c32[i * TQ // 2:(i + 1) * TQ // 2, :])
        r = slice(i * TQ // 2, (i + 1) * TQ // 2)
        kv32[0, r, :] = _pack(_nn(cc, wuk).astype(bf16))
        kv32[1, r, :] = _pack(_nn(cc, wuv).astype(bf16))

    def qproj(i, wq):
        return (_nn(_unpack(x32[i * TQ // 2:(i + 1) * TQ // 2, :]), wq) * QSCALE).astype(bf16)

    def scores(q, h, w):
        mask = col <= row
        k = _unpack(kv32[0, 0:w // 2, h * D:(h + 1) * D])
        s1 = _nt(q, k[0:w - T])
        s2 = _nt(q[T:], k[w - T:w])
        top_d = jnp.where(mask, s1[:T, w - 2 * T:], NEG)
        top = jnp.concatenate([s1[:T, :w - 2 * T], top_d], axis=1) if w > 2 * T else top_d
        bot = jnp.concatenate([s1[T:, :], jnp.where(mask, s2, NEG)], axis=1)
        return top, bot

    def probs(sc, w):
        top, bot = sc
        pt = jnp.exp2(top - jnp.max(top, axis=1, keepdims=True))
        pb = jnp.exp2(bot - jnp.max(bot, axis=1, keepdims=True))
        pk = (lax.bitcast_convert_type(pt, u32) >> 16) | (
            lax.bitcast_convert_type(pb[:, :w - T], u32) & u32(0xFFFF0000))
        return pk, pb[:, w - T:].astype(bf16)

    def pv(sc, h, w, defer=False):
        pk, pl_ = probs(sc, w)
        v = _unpack(kv32[1, 0:w // 2, h * D:(h + 1) * D])
        o1 = _nn(_unpack(pk), v[0:w - T])
        o2 = _nn(pl_, v[w - T:w])
        lo = lax.bitcast_convert_type(pk << 16, f32)
        hi = lax.bitcast_convert_type(pk & u32(0xFFFF0000), f32)
        lt = jnp.sum(lo, axis=1, keepdims=True)
        lb = jnp.sum(jnp.concatenate([hi, pl_.astype(f32)], axis=1), axis=1, keepdims=True)
        osc[h] = o1
        if defer:
            dsc[0] = o2
            dsc[1] = jnp.broadcast_to(lt, (T, D))
            dsc[2] = jnp.broadcast_to(lb, (T, D))
            return None
        return pv_finish(h, o2, lt, lb)

    def pv_finish(h, o2, lt, lb):
        ot = osc[h, pl.ds(0, T, stride=2), :] * _recip(lt)
        ob = (osc[h, pl.ds(1, T, stride=2), :] + o2) * _recip(lb)
        return jnp.concatenate([ot, ob], axis=0).astype(bf16)

    def combine(i, a):
        rows = slice(i * TQ, (i + 1) * TQ)
        g = gbuf[rows, :]
        for jj in range(NJ):
            b = bbuf[jj, rows, :]
            obuf[rows, jj * T:(jj + 1) * T] = (b + g * (a[:, jj * T:(jj + 1) * T] - b)).astype(bf16)

    def oproj(i, ctx2, wo, final=False):
        rows = slice(i * TQ, (i + 1) * TQ)
        a = _nn(ctx2, wo) + acc[rows, :]
        if final:
            combine(i, a)
        else:
            acc[rows, :] = a

    def load_wo(s):
        return wo_s[pl.ds(2 * s, 2)].reshape(2 * D, M)

    def b_piece(s, a, prev):
        j = s // 2
        jl = pl.ds(_aligned(j * T, T), T)
        rows = slice(a * T, (a + 1) * T)
        taps = par_s[pl.ds(_aligned(j * 8, 8), 8), :]
        kf = bk_s[rows, jl].astype(f32)
        ks = kf * taps[0:1, :]
        tail = prev[1] if prev is not None else jnp.zeros((8, T), f32)
        ext = jnp.concatenate([tail, kf], axis=0)
        for t in range(1, KS):
            ks = ks + pltpu.roll(ext, t, 0)[8:, :] * taps[t:t + 1, :]
        u = ks * bv_s[rows, jl].astype(f32)
        ut[rows, :] = u * taps[KS:KS + 1, :]
        fm = f_s[s % 2]
        uh = _nn(fm, u.astype(bf16))
        ur, ui = uh[0:hf], uh[hf:T]
        bst[0, a] = ur
        bst[1, a] = ui
        bst[2, a] = ur + ui
        hh = _nt(fm, sk_s[pl.ds(_aligned(j * T, T), T), rows])
        hr, hi = hh[0:hf], hh[hf:T]
        if prev is not None:
            prev_h = prev[0]
            pr, pi = prev_h[0:hf], prev_h[hf:T]
            q = hf // 2
            hr = jnp.concatenate([hr[:q] - pi[:q], hr[q:] + pi[q:]], axis=0)
            hi = jnp.concatenate([hi[:q] + pr[:q], hi[q:] - pr[q:]], axis=0)
        bst[3, a] = hr
        bst[4, a] = hi - hr
        bst[5, a] = hr + hi
        return hh, kf[T - 8:, :]

    def b_front(s):
        ph = None
        for a in range(NC):
            ph = b_piece(s, a, ph)

    def b_mac(s, c, last=False):
        k1 = k2 = k3 = None
        for a in range(c + 1):
            jj = c - a
            t1 = bst[3, jj] * bst[2, a]
            t2 = bst[0, a] * bst[4, jj]
            t3 = bst[1, a] * bst[5, jj]
            k1 = t1 if k1 is None else k1 + t1
            k2 = t2 if k2 is None else k2 + t2
            k3 = t3 if k3 is None else k3 + t3
        z = jnp.concatenate([k1 - k3, k1 + k2], axis=0).astype(bf16)
        rows = slice(c * T, (c + 1) * T)
        y = _nn(gi_s[s % 2], z)
        if last:
            y = y + ybuf[rows, :]
        else:
            y = y + jnp.where(s % 2 == 1, ybuf[rows, :], 0.0)
            ybuf[rows, :] = y
        j = s // 2
        jl = pl.ds(_aligned(j * T, T), T)
        bbuf[j, rows, :] = x_s[rows, jl].astype(f32) * (y + ut[rows, :])

    def front_first():
        cp_w(1, 0).start()
        cp_w(2, 0).start()
        for i in range(NCC):
            cp_c(i).start()
        for i in range(5):
            cp_small(i).start()
        cp_w(0, 0).start()
        cp_x(NB - 1).start()
        for kind in range(3):
            cp_b(kind, 0).start()
        for i in range(NB - 2, 1, -1):
            cp_x(i).start()
        cp_wo(0).start()
        cp_x(1).start()
        cp_x(0).start()
        cp_wo(1).start()
        for kind in range(3):
            cp_w(kind, 1).start()
        for kind in range(3):
            cp_b(kind, 1).start()
        cp_wo(2).start()
        for g in range(2, NG):
            for kind in range(3):
                cp_w(kind, g).start()

        def zero(i, carry):
            acc[pl.ds(pl.multiple_of(i * 64, 64), 64), :] = jnp.zeros((64, M), f32)
            return carry

        lax.fori_loop(0, S // 64, zero, 0)
        cp_w(1, 0).wait()
        convert_loop(1)
        cp_w(2, 0).wait()
        convert_loop(2)
        rc = S // NCC

        def kv_chunk(i, carry):
            r = pl.ds(pl.multiple_of(i * rc, rc), rc)
            pltpu.make_async_copy(c_hbm.at[r, :], c_s.at[r, :], sems.at[SEM_C + i]).wait()
            cc = c_s[r, :]
            rp = pl.ds(pl.multiple_of(i * (rc // 2), rc // 2), rc // 2)
            c32[rp, :] = _pack(cc)
            kv32[0, rp, :] = _pack(_nn(cc, load_w(1, 0)).astype(bf16))
            kv32[1, rp, :] = _pack(_nn(cc, load_w(2, 0)).astype(bf16))
            return carry

        lax.fori_loop(0, NCC, kv_chunk, 0)
        cp_w(0, 0).wait()
        convert_loop(0)
        for i in range(5):
            cp_small(i).wait()
        x_ready(NB - 1)
        qa32[...] = _pack(qproj(NB - 1, load_w(0, 0)))
        for kind in range(3):
            cp_b(kind, 0).wait()
        shf = sh_s[...].astype(f32)
        sdf = sd_s[...].astype(f32).reshape(1, M)
        for jj in range(NJ):
            par_s[jj * 8:jj * 8 + KS, :] = shf[:, jj * T:(jj + 1) * T]
            par_s[jj * 8 + KS:jj * 8 + KS + 1, :] = sdf[:, jj * T:(jj + 1) * T]
            par_s[jj * 8 + KS + 1:jj * 8 + 8, :] = jnp.zeros((8 - KS - 1, T), f32)
        b_front(0)
        x_ready_loop(NB - 2, NB - 3)
        cp_wo(0).wait()

    def seg_a(s):
        wq = load_w(0, s)
        wo = load_wo(s)
        qn = _unpack(qa32[...])
        prev = None
        for i in range(NB - 1, SPLIT - 1, -1):
            w = (i + 1) * TQ
            q2 = qn
            sc = [None, None]
            ctx = [None, None]
            for op in ORDER_A[i].split("."):
                if op == "SA":
                    sc[0] = scores(q2[:, 0:D], 0, w)
                elif op == "SB":
                    sc[1] = scores(q2[:, D:2 * D], 1, w)
                elif op[0] == "M":
                    b_mac(s, int(op[1:]))
                elif op == "Q":
                    qn = qproj(i - 1, wq)
                elif op == "PA":
                    ctx[0] = pv(sc[0], 0, w)
                elif op == "PB":
                    ctx[1] = pv(sc[1], 1, w, defer=(i == SPLIT))
                    if ctx[1] is None:
                        ctx[1] = ctx[0]
                elif op == "O":
                    if prev is not None:
                        oproj(i + 1, prev, wo)
            prev = jnp.concatenate(ctx, axis=1)
        qb32[...] = _pack(qn)
        cx32[...] = _pack(prev)

    def seg_b(s, last):
        if not last:
            sn = s + 1
            gsrc = jnp.minimum(s // P + 1, NG - 1)
            gdst = s // P + 1
            q4 = s % P
            for kind in range(3):
                n = w_rows[kind] // P
                convert(kind, gsrc, gdst, _aligned(q4 * n, n), n)
            wuk = load_w(1, sn)
            wuv = load_w(2, sn)
        wq = load_w(0, s)
        wo = load_wo(s)
        st = {"q": _unpack(qb32[...]), "prev": _unpack(cx32[...]), "h": None, "a": 0}
        st["prev"] = jnp.concatenate([st["prev"][:, 0:D], pv_finish(1, dsc[0], dsc[1], dsc[2])], axis=1)

        def job(name):
            kind, i = name[0], int(name[-1])
            if name[0] == "M":
                b_mac(s, i, last)
            elif name[:2] in ("SA", "SB"):
                h = 0 if name[1] == "A" else 1
                st["sc", h] = scores(st["q", i][:, h * D:(h + 1) * D], h, (i + 1) * TQ)
            elif kind == "Q":
                st["q", i] = qproj(i, wq)
            elif name[:2] in ("PA", "PB"):
                h = 0 if name[1] == "A" else 1
                st["ctx", i, h] = pv(st["sc", h], h, (i + 1) * TQ)
            elif kind == "O":
                ctx = st["prev"] if i == SPLIT else jnp.concatenate([st["ctx", i, 0], st["ctx", i, 1]], axis=1)
                oproj(i, ctx, wo, last)
            elif kind == "K":
                if not last:
                    kvproj(i, wuk, wuv)
            elif kind == "N":
                if not last:
                    qa32[...] = _pack(qproj(NB - 1, load_w(0, sn)))
            elif kind == "C":
                if last:
                    combine(i, acc[i * TQ:(i + 1) * TQ, :])
            elif kind == "D":
                if last:
                    cp_out(i).start()
            elif kind == "F":
                if not last:
                    for _ in range(i):
                        if st["a"] < NC:
                            st["h"] = b_piece(sn, st["a"], st["h"])
                            st["a"] += 1

        st["q", SPLIT - 1] = st["q"]
        jobs = (ORDER_LAST if last else ORDER_B).split(".")
        for name in jobs:
            job(name)
        if not last:
            assert st["a"] == NC, st["a"]
        else:
            for k in range(len(OUT_CHUNKS)):
                cp_out(k).wait()


    front_first()

    def step(s, carry):
        seg_a(s)

        @pl.when(jnp.logical_and(s <= (NG - 2) * P, jnp.logical_or(s <= 1, s % P == 0)))
        def _():
            @pl.when(s == 0)
            def _():
                x_ready_loop(1, 2)
                cp_wo(1).wait()
                for kind in range(3):
                    cp_w(kind, 1).wait()

            @pl.when(s == 1)
            def _():
                cp_wo(2).wait()
                for kind in range(3):
                    cp_b(kind, 1).wait()

            for g in range(2, NG):
                @pl.when(s == (g - 1) * P)
                def _():
                    for kind in range(3):
                        cp_w(kind, g).wait()

        @pl.when(s < NS - 1)
        def _():
            seg_b(s, False)

        @pl.when(s == NS - 1)
        def _():
            seg_b(s, True)

        return carry

    lax.fori_loop(0, NS, step, 0)


@jax.jit
def pallas_gated_mix__compressed_kv_cla__ssm_conv_h3__prompt_kernel(
    A_x: jax.Array,
    A_c_kv: jax.Array,
    A_w_q: jax.Array,
    A_w_uk: jax.Array,
    A_w_uv: jax.Array,
    A_w_o: jax.Array,
    B_q: jax.Array,
    B_k: jax.Array,
    B_v: jax.Array,
    B_shift_k: jax.Array,
    B_ssm_k: jax.Array,
    B_ssm_D: jax.Array,
    gate_w: jax.Array,
):
    del B_q
    x = A_x.reshape(S, M)
    c = A_c_kv.reshape(S, C)
    bk = B_k.reshape(S, M)
    bv = B_v.reshape(S, M)
    sh = B_shift_k.T
    fwd, inv = _dft_tables()
    fwd = jnp.asarray(fwd, dtype=bf16)
    inv = jnp.asarray(inv, dtype=bf16)

    any_spec = pl.BlockSpec(memory_space=pl.ANY)
    out = pl.pallas_call(
        _kernel,
        in_specs=[any_spec] * 14,
        out_specs=any_spec,
        out_shape=jax.ShapeDtypeStruct((S, M), bf16),
        scratch_shapes=[
            pltpu.VMEM((S, M), bf16),
            pltpu.VMEM((S, C), bf16),
            pltpu.VMEM((NG, M, G, D), bf16),
            pltpu.VMEM((NG, C, G, D), bf16),
            pltpu.VMEM((NG, C, G, D), bf16),
            pltpu.VMEM((NG + 1, M * P, D), u32),
            pltpu.VMEM((NG + 1, C * P, D), u32),
            pltpu.VMEM((NG + 1, C * P, D), u32),
            pltpu.VMEM((H, D, M), bf16),
            pltpu.VMEM((S, M), bf16),
            pltpu.VMEM((S, M), bf16),
            pltpu.VMEM((M, S), bf16),
            pltpu.VMEM((KS, M), bf16),
            pltpu.VMEM((M,), bf16),
            pltpu.VMEM((M,), bf16),
            pltpu.VMEM((2, T, T), bf16),
            pltpu.VMEM((2, T, T), bf16),
            pltpu.VMEM((NJ * 8, T), f32),
            pltpu.VMEM((2, S // 2, 2 * D), u32),
            pltpu.VMEM((TQ // 2, 2 * D), u32),
            pltpu.VMEM((TQ // 2, 2 * D), u32),
            pltpu.VMEM((TQ // 2, 2 * D), u32),
            pltpu.VMEM((6, NC, T // 2, T), f32),
            pltpu.VMEM((S, T), f32),
            pltpu.VMEM((2, TQ, D), f32),
            pltpu.VMEM((S // 2, M), u32),
            pltpu.VMEM((S // 2, C), u32),
            pltpu.VMEM((3, T, D), f32),
            pltpu.VMEM((S, M), f32),
            pltpu.VMEM((S, T), f32),
            pltpu.VMEM((NJ, S, T), f32),
            pltpu.VMEM((S, T), f32),
            pltpu.VMEM((S, M), bf16),
            pltpu.SemaphoreType.DMA((NSEM,)),
        ],
        compiler_params=pltpu.CompilerParams(
            vmem_limit_bytes=120 * 1024 * 1024,
        ),
        name="gated_mix",
    )(x, c, A_w_q, A_w_uk, A_w_uv, A_w_o, bk, bv, B_ssm_k, sh, B_ssm_D, gate_w, fwd, inv)
    return out.reshape(1, S, M)
```

```python
import numpy as np
import jax
import jax.numpy as jnp
from jax import lax
import jax.experimental.pallas as pl
import jax.experimental.pallas.tpu as pltpu

S, M, H, D, C = 2048, 1024, 32, 128, 512
G = 8
P = G // 2
NG = H // G
NS = H // 2
T = 128
TQ = 256
NB = S // TQ
NC = S // T
NJ = M // T
KS = 4
SPLIT = 3
NEG = -1e9
OUT_CHUNKS = [(7, 7), (5, 6), (3, 4), (2, 2), (1, 1), (0, 0)]
QSCALE = float(D ** -0.5 * np.log2(np.e))
bf16 = jnp.bfloat16
f32 = jnp.float32
u32 = jnp.uint32

ORDER_A = {7: "SA.SB.Q.M15.PA.O.M4.PB", 6: "SA.SB.Q.M14.PA.O.M5.PB", 5: "SA.SB.Q.M13.PA.O.M6.PB",
           4: "SA.SB.Q.M12.PA.O.M7.M8.PB", 3: "SA.Q.SB.M11.PA.O.M10.M9.PB"}
ORDER_B = ("SA2.SB2.Q1.M3.M2.M1.M0.PA2.F1.O3.F1.K7.F1.PB2.F1.K6.F1.SA1.F1.SB1.F1.Q0.F1.PA1.F1.O2.F1."
           "K5.F1.PB1.F1.K4.F1.K2.F1.SA0.SB0.K3.F1.PA0.O1.F1.PB0.K1.F1.O0.F1.K0.N0")
ORDER_LAST = ("SA2.C7.D0.SB2.C6.Q1.C5.D1.M3.M2.M1.M0.PA2.C4.O3.D2.PB2.SA1.SB1.Q0.PA1.O2.D3."
              "PB1.SA0.SB0.PA0.O1.D4.PB0.O0.D5")

NCC = 4
SEM_C = 0
SEM_X = SEM_C + NCC
SEM_W = SEM_X + NB
SEM_WO = SEM_W + 3 * NG
SEM_B = SEM_WO + 3
SEM_S = SEM_B + 6
SEM_P = SEM_S + 5
SEM_O = SEM_P + 3
NSEM = SEM_O + len(OUT_CHUNKS)


def _nt(a, b):
    return lax.dot_general(a, b, (((1,), (1,)), ((), ())), preferred_element_type=f32)


def _nn(a, b):
    return jnp.dot(a, b, preferred_element_type=f32)


def _pack(v):
    return pltpu.bitcast(v, u32)


def _unpack(v):
    return pltpu.bitcast(v, bf16)


def _unpack_pair(w32):
    lo = lax.bitcast_convert_type(w32 << 16, f32).astype(bf16)
    hi = lax.bitcast_convert_type(w32 & u32(0xFFFF0000), f32).astype(bf16)
    return jnp.concatenate([lo, hi], axis=1)


def _recip(l):
    r = pl.reciprocal(l, approx=True)
    return r * (2.0 - l * r)


def _aligned(v, n):
    return v if isinstance(v, int) else pl.multiple_of(v, n)


def _dft_tables():
    n = np.arange(T)[None, :]
    k = np.arange(T)[:, None]
    ang = 2.0 * np.pi * ((n * (2 * k + 1)) % (4 * T)) / (4 * T)
    cos, sin = np.cos(ang), np.sin(ang)
    hf = T // 2
    halves = []
    for h in range(2):
        ks = np.arange(h * hf, (h + 1) * hf)
        ks = np.concatenate([ks[0::2], ks[1::2]])
        halves.append(np.concatenate([cos[ks], -sin[ks]], axis=0))
    fwd = np.stack(halves)
    inv = np.transpose(fwd, (0, 2, 1)) / T
    return fwd.astype(np.float32), inv.astype(np.float32)


def _kernel(x_hbm, c_hbm, wq_hbm, wuk_hbm, wuv_hbm, wo_hbm, bk_hbm, bv_hbm, sk_hbm,
            sh_hbm, sd_hbm, gw_hbm, f_hbm, gi_hbm,
            o_hbm,
            x_s, c_s, wq_b, wuk_b, wuv_b, wq32, wuk32, wuv32, wo_s, bk_s, bv_s, sk_s,
            sh_s, sd_s, gw_s, f_s, gi_s, par_s,
            kv32, qa32, qb32, cx32, bst, ut, osc, x32, c32, dsc,
            acc, ybuf, bbuf, gbuf, obuf, sems):
    def cp(src, dst, sem):
        return pltpu.make_async_copy(src, dst, sems.at[sem])

    def cp_c(i):
        r = pl.ds(i * (S // NCC), S // NCC)
        return cp(c_hbm.at[r, :], c_s.at[r, :], SEM_C + i)

    def cp_x(i):
        r = pl.ds(i * TQ, TQ)
        return cp(x_hbm.at[r, :], x_s.at[r, :], SEM_X + i)

    w_hbm = (wq_hbm, wuk_hbm, wuv_hbm)
    w_b = (wq_b, wuk_b, wuv_b)
    w_32 = (wq32, wuk32, wuv32)
    w_rows = (M, C, C)

    def cp_w(kind, g):
        return cp(w_hbm[kind].at[:, pl.ds(g * G, G), :], w_b[kind].at[g], SEM_W + kind * NG + g)

    def cp_pair0(kind):
        return cp(w_hbm[kind].at[:, pl.ds(0, 2), :], w_b[kind].at[0, :, pl.ds(0, 2), :], SEM_P + kind)

    def zero_group0(kind):
        def body(c, carry):
            w_b[kind][0, pl.ds(pl.multiple_of(c * 64, 64), 64), :, :] = jnp.zeros((64, G, D), bf16)
            return carry

        lax.fori_loop(0, w_rows[kind] // 64, body, 0)

    def cp_wo(part):
        r = (pl.ds(0, 2), pl.ds(2, 2), pl.ds(4, H - 4))[part]
        return cp(wo_hbm.at[r], wo_s.at[r], SEM_WO + part)

    def cp_b(kind, part):
        r = (pl.ds(0, T), pl.ds(T, M - T))[part]
        if kind == 2:
            return cp(sk_hbm.at[r, :], sk_s.at[r, :], SEM_B + 2 * kind + part)
        src, dst = ((bk_hbm, bk_s), (bv_hbm, bv_s))[kind]
        return cp(src.at[:, r], dst.at[:, r], SEM_B + 2 * kind + part)

    def cp_small(i):
        src, dst = ((sh_hbm, sh_s), (sd_hbm, sd_s), (gw_hbm, gw_s), (f_hbm, f_s), (gi_hbm, gi_s))[i]
        return cp(src, dst, SEM_S + i)

    def cp_out(k):
        lo, hi = OUT_CHUNKS[k]
        r = pl.ds(lo * TQ, (hi - lo + 1) * TQ)
        return cp(obuf.at[r, :], o_hbm.at[r, :], SEM_O + k)

    def convert(kind, g_src, g_dst, r0, nrows):
        ch = 64
        for c0 in range(0, nrows, ch):
            v = w_b[kind][g_src, pl.ds(r0 + c0, ch), :, :]
            w_32[kind][g_dst, pl.ds((r0 + c0) * P, ch * P), :] = _pack(v.reshape(ch * G, D))

    def convert_loop(kind):
        def body(c, carry):
            convert(kind, 0, 0, pl.multiple_of(c * 64, 64), 64)
            return carry

        lax.fori_loop(0, w_rows[kind] // 64, body, 0)

    def x_ready(i):
        r = pl.ds(_aligned(i * TQ, TQ), TQ)
        pltpu.make_async_copy(x_hbm.at[r, :], x_s.at[r, :], sems.at[SEM_X + i]).wait()
        xv = x_s[r, :]
        x32[pl.ds(_aligned(i * (TQ // 2), TQ // 2), TQ // 2), :] = _pack(xv)
        z = jnp.sum(xv.astype(f32) * gw_s[...].astype(f32).reshape(1, M), axis=1, keepdims=True)
        gbuf[r, :] = jnp.broadcast_to(1.0 / (1.0 + jnp.exp(-z)), (TQ, T))

    def x_ready_loop(first, count):
        def body(t, carry):
            x_ready(first - t)
            return carry

        lax.fori_loop(0, count, body, 0)

    def load_w(kind, s):
        return _unpack_pair(w_32[kind][s // P, pl.ds(s % P, w_rows[kind], stride=P), :])

    row = lax.broadcasted_iota(jnp.int32, (T, T), 0)
    col = lax.broadcasted_iota(jnp.int32, (T, T), 1)
    hf = T // 2

    def kvproj(i, wuk, wuv):
        cc = _unpack(c32[i * TQ // 2:(i + 1) * TQ // 2, :])
        r = slice(i * TQ // 2, (i + 1) * TQ // 2)
        kv32[0, r, :] = _pack(_nn(cc, wuk).astype(bf16))
        kv32[1, r, :] = _pack(_nn(cc, wuv).astype(bf16))

    def qproj(i, wq):
        return (_nn(_unpack(x32[i * TQ // 2:(i + 1) * TQ // 2, :]), wq) * QSCALE).astype(bf16)

    def scores(q, h, w):
        mask = col <= row
        k = _unpack(kv32[0, 0:w // 2, h * D:(h + 1) * D])
        s1 = _nt(q, k[0:w - T])
        s2 = _nt(q[T:], k[w - T:w])
        top_d = jnp.where(mask, s1[:T, w - 2 * T:], NEG)
        top = jnp.concatenate([s1[:T, :w - 2 * T], top_d], axis=1) if w > 2 * T else top_d
        bot = jnp.concatenate([s1[T:, :], jnp.where(mask, s2, NEG)], axis=1)
        return top, bot

    def probs(sc, w):
        top, bot = sc
        pt = jnp.exp2(top - jnp.max(top, axis=1, keepdims=True))
        pb = jnp.exp2(bot - jnp.max(bot, axis=1, keepdims=True))
        pk = (lax.bitcast_convert_type(pt, u32) >> 16) | (
            lax.bitcast_convert_type(pb[:, :w - T], u32) & u32(0xFFFF0000))
        return pk, pb[:, w - T:].astype(bf16)

    def pv(sc, h, w, defer=False):
        pk, pl_ = probs(sc, w)
        v = _unpack(kv32[1, 0:w // 2, h * D:(h + 1) * D])
        o1 = _nn(_unpack(pk), v[0:w - T])
        o2 = _nn(pl_, v[w - T:w])
        lo = lax.bitcast_convert_type(pk << 16, f32)
        hi = lax.bitcast_convert_type(pk & u32(0xFFFF0000), f32)
        lt = jnp.sum(lo, axis=1, keepdims=True)
        lb = jnp.sum(jnp.concatenate([hi, pl_.astype(f32)], axis=1), axis=1, keepdims=True)
        osc[h] = o1
        if defer:
            dsc[0] = o2
            dsc[1] = jnp.broadcast_to(lt, (T, D))
            dsc[2] = jnp.broadcast_to(lb, (T, D))
            return None
        return pv_finish(h, o2, lt, lb)

    def pv_finish(h, o2, lt, lb):
        ot = osc[h, pl.ds(0, T, stride=2), :] * _recip(lt)
        ob = (osc[h, pl.ds(1, T, stride=2), :] + o2) * _recip(lb)
        return jnp.concatenate([ot, ob], axis=0).astype(bf16)

    def combine(i, a):
        rows = slice(i * TQ, (i + 1) * TQ)
        g = gbuf[rows, :]
        for jj in range(NJ):
            b = bbuf[jj, rows, :]
            obuf[rows, jj * T:(jj + 1) * T] = (b + g * (a[:, jj * T:(jj + 1) * T] - b)).astype(bf16)

    def oproj(i, ctx2, wo, final=False):
        rows = slice(i * TQ, (i + 1) * TQ)
        a = _nn(ctx2, wo) + acc[rows, :]
        if final:
            combine(i, a)
        else:
            acc[rows, :] = a

    def load_wo(s):
        return wo_s[pl.ds(2 * s, 2)].reshape(2 * D, M)

    def b_piece(s, a, prev):
        j = s // 2
        jl = pl.ds(_aligned(j * T, T), T)
        rows = slice(a * T, (a + 1) * T)
        taps = par_s[pl.ds(_aligned(j * 8, 8), 8), :]
        kf = bk_s[rows, jl].astype(f32)
        ks = kf * taps[0:1, :]
        tail = prev[1] if prev is not None else jnp.zeros((8, T), f32)
        ext = jnp.concatenate([tail, kf], axis=0)
        for t in range(1, KS):
            ks = ks + pltpu.roll(ext, t, 0)[8:, :] * taps[t:t + 1, :]
        u = ks * bv_s[rows, jl].astype(f32)
        ut[rows, :] = u * taps[KS:KS + 1, :]
        fm = f_s[s % 2]
        uh = _nn(fm, u.astype(bf16))
        ur, ui = uh[0:hf], uh[hf:T]
        bst[0, a] = ur
        bst[1, a] = ui
        bst[2, a] = ur + ui
        hh = _nt(fm, sk_s[pl.ds(_aligned(j * T, T), T), rows])
        hr, hi = hh[0:hf], hh[hf:T]
        if prev is not None:
            prev_h = prev[0]
            pr, pi = prev_h[0:hf], prev_h[hf:T]
            q = hf // 2
            hr = jnp.concatenate([hr[:q] - pi[:q], hr[q:] + pi[q:]], axis=0)
            hi = jnp.concatenate([hi[:q] + pr[:q], hi[q:] - pr[q:]], axis=0)
        bst[3, a] = hr
        bst[4, a] = hi - hr
        bst[5, a] = hr + hi
        return hh, kf[T - 8:, :]

    def b_front(s):
        ph = None
        for a in range(NC):
            ph = b_piece(s, a, ph)

    def b_mac(s, c, last=False):
        k1 = k2 = k3 = None
        for a in range(c + 1):
            jj = c - a
            t1 = bst[3, jj] * bst[2, a]
            t2 = bst[0, a] * bst[4, jj]
            t3 = bst[1, a] * bst[5, jj]
            k1 = t1 if k1 is None else k1 + t1
            k2 = t2 if k2 is None else k2 + t2
            k3 = t3 if k3 is None else k3 + t3
        z = jnp.concatenate([k1 - k3, k1 + k2], axis=0).astype(bf16)
        rows = slice(c * T, (c + 1) * T)
        y = _nn(gi_s[s % 2], z)
        if last:
            y = y + ybuf[rows, :]
        else:
            y = y + jnp.where(s % 2 == 1, ybuf[rows, :], 0.0)
            ybuf[rows, :] = y
        j = s // 2
        jl = pl.ds(_aligned(j * T, T), T)
        bbuf[j, rows, :] = x_s[rows, jl].astype(f32) * (y + ut[rows, :])

    def front_first():
        cp_c(0).start()
        for kind in (1, 2):
            zero_group0(kind)
            cp_pair0(kind).start()
        for i in range(1, NCC):
            cp_c(i).start()
        for i in range(5):
            cp_small(i).start()
        cp_x(NB - 1).start()
        for kind in range(3):
            cp_b(kind, 0).start()
        zero_group0(0)
        cp_pair0(0).start()
        for i in range(NB - 2, 1, -1):
            cp_x(i).start()
        cp_wo(0).start()
        cp_x(1).start()
        cp_x(0).start()

        cp_pair0(1).wait()
        convert_loop(1)
        cp_pair0(2).wait()
        convert_loop(2)
        cp_w(1, 0).start()
        cp_w(2, 0).start()
        rc = S // NCC

        def kv_chunk(i, carry):
            r = pl.ds(pl.multiple_of(i * rc, rc), rc)
            pltpu.make_async_copy(c_hbm.at[r, :], c_s.at[r, :], sems.at[SEM_C + i]).wait()
            cc = c_s[r, :]
            rp = pl.ds(pl.multiple_of(i * (rc // 2), rc // 2), rc // 2)
            c32[rp, :] = _pack(cc)
            kv32[0, rp, :] = _pack(_nn(cc, load_w(1, 0)).astype(bf16))
            kv32[1, rp, :] = _pack(_nn(cc, load_w(2, 0)).astype(bf16))
            acc[r, :] = jnp.zeros((rc, M), f32)
            return carry

        lax.fori_loop(0, NCC, kv_chunk, 0)
        cp_pair0(0).wait()
        convert_loop(0)
        cp_w(0, 0).start()
        cp_wo(1).start()
        for kind in range(3):
            cp_w(kind, 1).start()
        for kind in range(3):
            cp_b(kind, 1).start()
        cp_wo(2).start()
        for g in range(2, NG):
            for kind in range(3):
                cp_w(kind, g).start()
        for i in range(5):
            cp_small(i).wait()
        x_ready(NB - 1)
        qa32[...] = _pack(qproj(NB - 1, load_w(0, 0)))
        for kind in range(3):
            cp_b(kind, 0).wait()
        shf = sh_s[...].astype(f32)
        sdf = sd_s[...].astype(f32).reshape(1, M)
        for jj in range(NJ):
            par_s[jj * 8:jj * 8 + KS, :] = shf[:, jj * T:(jj + 1) * T]
            par_s[jj * 8 + KS:jj * 8 + KS + 1, :] = sdf[:, jj * T:(jj + 1) * T]
            par_s[jj * 8 + KS + 1:jj * 8 + 8, :] = jnp.zeros((8 - KS - 1, T), f32)
        b_front(0)
        x_ready_loop(NB - 2, NB - 3)
        cp_wo(0).wait()

    def seg_a(s):
        wq = load_w(0, s)
        wo = load_wo(s)
        qn = _unpack(qa32[...])
        prev = None
        for i in range(NB - 1, SPLIT - 1, -1):
            w = (i + 1) * TQ
            q2 = qn
            sc = [None, None]
            ctx = [None, None]
            for op in ORDER_A[i].split("."):
                if op == "SA":
                    sc[0] = scores(q2[:, 0:D], 0, w)
                elif op == "SB":
                    sc[1] = scores(q2[:, D:2 * D], 1, w)
                elif op[0] == "M":
                    b_mac(s, int(op[1:]))
                elif op == "Q":
                    qn = qproj(i - 1, wq)
                elif op == "PA":
                    ctx[0] = pv(sc[0], 0, w)
                elif op == "PB":
                    ctx[1] = pv(sc[1], 1, w, defer=(i == SPLIT))
                    if ctx[1] is None:
                        ctx[1] = ctx[0]
                elif op == "O":
                    if prev is not None:
                        oproj(i + 1, prev, wo)
            prev = jnp.concatenate(ctx, axis=1)
        qb32[...] = _pack(qn)
        cx32[...] = _pack(prev)

    def seg_b(s, last):
        if not last:
            sn = s + 1
            gsrc = jnp.minimum(s // P + 1, NG - 1)
            gdst = s // P + 1
            q4 = s % P
            for kind in range(3):
                n = w_rows[kind] // P
                convert(kind, gsrc, gdst, _aligned(q4 * n, n), n)
            wuk = load_w(1, sn)
            wuv = load_w(2, sn)
        wq = load_w(0, s)
        wo = load_wo(s)
        st = {"q": _unpack(qb32[...]), "prev": _unpack(cx32[...]), "h": None, "a": 0}
        st["prev"] = jnp.concatenate([st["prev"][:, 0:D], pv_finish(1, dsc[0], dsc[1], dsc[2])], axis=1)

        def job(name):
            kind, i = name[0], int(name[-1])
            if name[0] == "M":
                b_mac(s, i, last)
            elif name[:2] in ("SA", "SB"):
                h = 0 if name[1] == "A" else 1
                st["sc", h] = scores(st["q", i][:, h * D:(h + 1) * D], h, (i + 1) * TQ)
            elif kind == "Q":
                st["q", i] = qproj(i, wq)
            elif name[:2] in ("PA", "PB"):
                h = 0 if name[1] == "A" else 1
                st["ctx", i, h] = pv(st["sc", h], h, (i + 1) * TQ)
            elif kind == "O":
                ctx = st["prev"] if i == SPLIT else jnp.concatenate([st["ctx", i, 0], st["ctx", i, 1]], axis=1)
                oproj(i, ctx, wo, last)
            elif kind == "K":
                if not last:
                    kvproj(i, wuk, wuv)
            elif kind == "N":
                if not last:
                    qa32[...] = _pack(qproj(NB - 1, load_w(0, sn)))
            elif kind == "C":
                if last:
                    combine(i, acc[i * TQ:(i + 1) * TQ, :])
            elif kind == "D":
                if last:
                    cp_out(i).start()
            elif kind == "F":
                if not last:
                    for _ in range(i):
                        if st["a"] < NC:
                            st["h"] = b_piece(sn, st["a"], st["h"])
                            st["a"] += 1

        st["q", SPLIT - 1] = st["q"]
        jobs = (ORDER_LAST if last else ORDER_B).split(".")
        for name in jobs:
            job(name)
        if not last:
            assert st["a"] == NC, st["a"]
        else:
            for k in range(len(OUT_CHUNKS)):
                cp_out(k).wait()


    front_first()

    def step(s, carry):
        seg_a(s)

        @pl.when(jnp.logical_and(s <= (NG - 2) * P, jnp.logical_or(s <= 1, s % P == 0)))
        def _():
            @pl.when(s == 0)
            def _():
                x_ready_loop(1, 2)
                for kind in range(3):
                    cp_w(kind, 0).wait()
                    convert_loop(kind)
                cp_wo(1).wait()
                for kind in range(3):
                    cp_w(kind, 1).wait()

            @pl.when(s == 1)
            def _():
                cp_wo(2).wait()
                for kind in range(3):
                    cp_b(kind, 1).wait()

            for g in range(2, NG):
                @pl.when(s == (g - 1) * P)
                def _():
                    for kind in range(3):
                        cp_w(kind, g).wait()

        @pl.when(s < NS - 1)
        def _():
            seg_b(s, False)

        @pl.when(s == NS - 1)
        def _():
            seg_b(s, True)

        return carry

    lax.fori_loop(0, NS, step, 0)


@jax.jit
def pallas_gated_mix__compressed_kv_cla__ssm_conv_h3__prompt_kernel(
    A_x: jax.Array,
    A_c_kv: jax.Array,
    A_w_q: jax.Array,
    A_w_uk: jax.Array,
    A_w_uv: jax.Array,
    A_w_o: jax.Array,
    B_q: jax.Array,
    B_k: jax.Array,
    B_v: jax.Array,
    B_shift_k: jax.Array,
    B_ssm_k: jax.Array,
    B_ssm_D: jax.Array,
    gate_w: jax.Array,
):
    del B_q
    x = A_x.reshape(S, M)
    c = A_c_kv.reshape(S, C)
    bk = B_k.reshape(S, M)
    bv = B_v.reshape(S, M)
    sh = B_shift_k.T
    fwd, inv = _dft_tables()
    fwd = jnp.asarray(fwd, dtype=bf16)
    inv = jnp.asarray(inv, dtype=bf16)

    any_spec = pl.BlockSpec(memory_space=pl.ANY)
    out = pl.pallas_call(
        _kernel,
        in_specs=[any_spec] * 14,
        out_specs=any_spec,
        out_shape=jax.ShapeDtypeStruct((S, M), bf16),
        scratch_shapes=[
            pltpu.VMEM((S, M), bf16),
            pltpu.VMEM((S, C), bf16),
            pltpu.VMEM((NG, M, G, D), bf16),
            pltpu.VMEM((NG, C, G, D), bf16),
            pltpu.VMEM((NG, C, G, D), bf16),
            pltpu.VMEM((NG + 1, M * P, D), u32),
            pltpu.VMEM((NG + 1, C * P, D), u32),
            pltpu.VMEM((NG + 1, C * P, D), u32),
            pltpu.VMEM((H, D, M), bf16),
            pltpu.VMEM((S, M), bf16),
            pltpu.VMEM((S, M), bf16),
            pltpu.VMEM((M, S), bf16),
            pltpu.VMEM((KS, M), bf16),
            pltpu.VMEM((M,), bf16),
            pltpu.VMEM((M,), bf16),
            pltpu.VMEM((2, T, T), bf16),
            pltpu.VMEM((2, T, T), bf16),
            pltpu.VMEM((NJ * 8, T), f32),
            pltpu.VMEM((2, S // 2, 2 * D), u32),
            pltpu.VMEM((TQ // 2, 2 * D), u32),
            pltpu.VMEM((TQ // 2, 2 * D), u32),
            pltpu.VMEM((TQ // 2, 2 * D), u32),
            pltpu.VMEM((6, NC, T // 2, T), f32),
            pltpu.VMEM((S, T), f32),
            pltpu.VMEM((2, TQ, D), f32),
            pltpu.VMEM((S // 2, M), u32),
            pltpu.VMEM((S // 2, C), u32),
            pltpu.VMEM((3, T, D), f32),
            pltpu.VMEM((S, M), f32),
            pltpu.VMEM((S, T), f32),
            pltpu.VMEM((NJ, S, T), f32),
            pltpu.VMEM((S, T), f32),
            pltpu.VMEM((S, M), bf16),
            pltpu.SemaphoreType.DMA((NSEM,)),
        ],
        compiler_params=pltpu.CompilerParams(
            vmem_limit_bytes=120 * 1024 * 1024,
        ),
        name="gated_mix",
    )(x, c, A_w_q, A_w_uk, A_w_uv, A_w_o, bk, bv, B_ssm_k, sh, B_ssm_D, gate_w, fwd, inv)
    return out.reshape(1, S, M)
```

```python
import numpy as np
import jax
import jax.numpy as jnp
from jax import lax
import jax.experimental.pallas as pl
import jax.experimental.pallas.tpu as pltpu

S, M, H, D, C = 2048, 1024, 32, 128, 512
G = 8
P = G // 2
NG = H // G
NS = H // 2
T = 128
TQ = 256
NB = S // TQ
NC = S // T
NJ = M // T
KS = 4
SPLIT = 3
NEG = -1e9
OUT_CHUNKS = [(7, 7), (5, 6), (3, 4), (2, 2), (1, 1), (0, 0)]
QSCALE = float(D ** -0.5 * np.log2(np.e))
bf16 = jnp.bfloat16
f32 = jnp.float32
u32 = jnp.uint32

ORDER_A = {7: "SA.SB.Q.M15.PA.O.M4.PB", 6: "SA.SB.Q.M14.PA.O.M5.PB", 5: "SA.SB.Q.M13.PA.O.M6.PB",
           4: "SA.SB.Q.M12.PA.O.M7.M8.PB", 3: "SA.Q.SB.M11.PA.O.M10.M9.PB"}
ORDER_B = ("SA2.SB2.Q1.M3.M2.M1.M0.PA2.F1.O3.F1.K7.F1.PB2.F1.K6.F1.SA1.F1.SB1.F1.Q0.F1.PA1.F1.O2.F1."
           "K5.F1.PB1.F1.K4.F1.K2.F1.SA0.SB0.K3.F1.PA0.O1.F1.PB0.K1.F1.O0.F1.K0.N0")
ORDER_LAST = ("SA2.C7.D0.SB2.C6.Q1.C5.D1.M3.M2.M1.M0.PA2.C4.O3.D2.PB2.SA1.SB1.Q0.PA1.O2.D3."
              "PB1.SA0.SB0.PA0.O1.D4.PB0.O0.D5")

NCC = 4
SEM_C = 0
SEM_X = SEM_C + NCC
SEM_W = SEM_X + NB
SEM_WO = SEM_W + 3 * NG
SEM_B = SEM_WO + 3
SEM_S = SEM_B + 6
SEM_P = SEM_S + 5
SEM_O = SEM_P + 3
NSEM = SEM_O + len(OUT_CHUNKS)


def _nt(a, b):
    return lax.dot_general(a, b, (((1,), (1,)), ((), ())), preferred_element_type=f32)


def _nn(a, b):
    return jnp.dot(a, b, preferred_element_type=f32)


def _pack(v):
    return pltpu.bitcast(v, u32)


def _unpack(v):
    return pltpu.bitcast(v, bf16)


def _unpack_pair(w32):
    lo = lax.bitcast_convert_type(w32 << 16, f32).astype(bf16)
    hi = lax.bitcast_convert_type(w32 & u32(0xFFFF0000), f32).astype(bf16)
    return jnp.concatenate([lo, hi], axis=1)


def _recip(l):
    r = pl.reciprocal(l, approx=True)
    return r * (2.0 - l * r)


def _aligned(v, n):
    return v if isinstance(v, int) else pl.multiple_of(v, n)


def _dft_tables():
    n = np.arange(T)[None, :]
    k = np.arange(T)[:, None]
    ang = 2.0 * np.pi * ((n * (2 * k + 1)) % (4 * T)) / (4 * T)
    cos, sin = np.cos(ang), np.sin(ang)
    hf = T // 2
    halves = []
    for h in range(2):
        ks = np.arange(h * hf, (h + 1) * hf)
        ks = np.concatenate([ks[0::2], ks[1::2]])
        halves.append(np.concatenate([cos[ks], -sin[ks]], axis=0))
    fwd = np.stack(halves)
    inv = np.transpose(fwd, (0, 2, 1)) / T
    return fwd.astype(np.float32), inv.astype(np.float32)


def _kernel(x_hbm, c_hbm, wq_hbm, wuk_hbm, wuv_hbm, wo_hbm, bk_hbm, bv_hbm, sk_hbm,
            sh_hbm, sd_hbm, gw_hbm, f_hbm, gi_hbm,
            o_hbm,
            x_s, c_s, wq_b, wuk_b, wuv_b, wq32, wuk32, wuv32, wo_s, bk_s, bv_s, sk_s,
            sh_s, sd_s, gw_s, f_s, gi_s, par_s,
            kv32, qa32, qb32, cx32, bst, ut, osc, x32, c32, dsc,
            acc, ybuf, bbuf, gbuf, obuf, sems):
    def cp(src, dst, sem):
        return pltpu.make_async_copy(src, dst, sems.at[sem])

    def cp_c(i):
        r = pl.ds(i * (S // NCC), S // NCC)
        return cp(c_hbm.at[r, :], c_s.at[r, :], SEM_C + i)

    def cp_x(i):
        r = pl.ds(i * TQ, TQ)
        return cp(x_hbm.at[r, :], x_s.at[r, :], SEM_X + i)

    w_hbm = (wq_hbm, wuk_hbm, wuv_hbm)
    w_b = (wq_b, wuk_b, wuv_b)
    w_32 = (wq32, wuk32, wuv32)
    w_rows = (M, C, C)

    def cp_w(kind, g):
        return cp(w_hbm[kind].at[:, pl.ds(g * G, G), :], w_b[kind].at[g], SEM_W + kind * NG + g)

    def cp_pair0(kind):
        return cp(w_hbm[kind].at[:, pl.ds(0, 2), :], w_b[kind].at[0, :, pl.ds(0, 2), :], SEM_P + kind)

    def zero_group0(kind):
        def body(c, carry):
            w_b[kind][0, pl.ds(pl.multiple_of(c * 64, 64), 64), :, :] = jnp.zeros((64, G, D), bf16)
            return carry

        lax.fori_loop(0, w_rows[kind] // 64, body, 0)

    def cp_wo(part):
        r = (pl.ds(0, 2), pl.ds(2, 2), pl.ds(4, H - 4))[part]
        return cp(wo_hbm.at[r], wo_s.at[r], SEM_WO + part)

    def cp_b(kind, part):
        r = (pl.ds(0, T), pl.ds(T, M - T))[part]
        if kind == 2:
            return cp(sk_hbm.at[r, :], sk_s.at[r, :], SEM_B + 2 * kind + part)
        src, dst = ((bk_hbm, bk_s), (bv_hbm, bv_s))[kind]
        return cp(src.at[:, r], dst.at[:, r], SEM_B + 2 * kind + part)

    def cp_small(i):
        src, dst = ((sh_hbm, sh_s), (sd_hbm, sd_s), (gw_hbm, gw_s), (f_hbm, f_s), (gi_hbm, gi_s))[i]
        return cp(src, dst, SEM_S + i)

    def cp_out(k):
        lo, hi = OUT_CHUNKS[k]
        r = pl.ds(lo * TQ, (hi - lo + 1) * TQ)
        return cp(obuf.at[r, :], o_hbm.at[r, :], SEM_O + k)

    def convert(kind, g_src, g_dst, r0, nrows):
        ch = 64
        for c0 in range(0, nrows, ch):
            v = w_b[kind][g_src, pl.ds(r0 + c0, ch), :, :]
            w_32[kind][g_dst, pl.ds((r0 + c0) * P, ch * P), :] = _pack(v.reshape(ch * G, D))

    def convert_loop(kind):
        def body(c, carry):
            convert(kind, 0, 0, pl.multiple_of(c * 64, 64), 64)
            return carry

        lax.fori_loop(0, w_rows[kind] // 64, body, 0)

    def x_ready(i):
        r = pl.ds(_aligned(i * TQ, TQ), TQ)
        pltpu.make_async_copy(x_hbm.at[r, :], x_s.at[r, :], sems.at[SEM_X + i]).wait()
        xv = x_s[r, :]
        x32[pl.ds(_aligned(i * (TQ // 2), TQ // 2), TQ // 2), :] = _pack(xv)
        z = jnp.sum(xv.astype(f32) * gw_s[...].astype(f32).reshape(1, M), axis=1, keepdims=True)
        gbuf[r, :] = jnp.broadcast_to(1.0 / (1.0 + jnp.exp(-z)), (TQ, T))

    def x_ready_loop(first, count):
        def body(t, carry):
            x_ready(first - t)
            return carry

        lax.fori_loop(0, count, body, 0)

    def load_w(kind, s):
        return _unpack_pair(w_32[kind][s // P, pl.ds(s % P, w_rows[kind], stride=P), :])

    row = lax.broadcasted_iota(jnp.int32, (T, T), 0)
    col = lax.broadcasted_iota(jnp.int32, (T, T), 1)
    hf = T // 2

    def kvproj(i, wuk, wuv):
        cc = _unpack(c32[i * TQ // 2:(i + 1) * TQ // 2, :])
        r = slice(i * TQ // 2, (i + 1) * TQ // 2)
        kv32[0, r, :] = _pack(_nn(cc, wuk).astype(bf16))
        kv32[1, r, :] = _pack(_nn(cc, wuv).astype(bf16))

    def qproj(i, wq):
        return (_nn(_unpack(x32[i * TQ // 2:(i + 1) * TQ // 2, :]), wq) * QSCALE).astype(bf16)

    def scores(q, h, w):
        mask = col <= row
        k = _unpack(kv32[0, 0:w // 2, h * D:(h + 1) * D])
        s1 = _nt(q, k[0:w - T])
        s2 = _nt(q[T:], k[w - T:w])
        top_d = jnp.where(mask, s1[:T, w - 2 * T:], NEG)
        top = jnp.concatenate([s1[:T, :w - 2 * T], top_d], axis=1) if w > 2 * T else top_d
        bot = jnp.concatenate([s1[T:, :], jnp.where(mask, s2, NEG)], axis=1)
        return top, bot

    def probs(sc, w):
        top, bot = sc
        pt = jnp.exp2(top - jnp.max(top, axis=1, keepdims=True))
        pb = jnp.exp2(bot - jnp.max(bot, axis=1, keepdims=True))
        pk = (lax.bitcast_convert_type(pt, u32) >> 16) | (
            lax.bitcast_convert_type(pb[:, :w - T], u32) & u32(0xFFFF0000))
        return pk, pb[:, w - T:].astype(bf16)

    def pv(sc, h, w, defer=False):
        pk, pl_ = probs(sc, w)
        v = _unpack(kv32[1, 0:w // 2, h * D:(h + 1) * D])
        o1 = _nn(_unpack(pk), v[0:w - T])
        o2 = _nn(pl_, v[w - T:w])
        lo = lax.bitcast_convert_type(pk << 16, f32)
        hi = lax.bitcast_convert_type(pk & u32(0xFFFF0000), f32)
        lt = jnp.sum(lo, axis=1, keepdims=True)
        lb = jnp.sum(jnp.concatenate([hi, pl_.astype(f32)], axis=1), axis=1, keepdims=True)
        osc[h] = o1
        if defer:
            dsc[0] = o2
            dsc[1] = jnp.broadcast_to(lt, (T, D))
            dsc[2] = jnp.broadcast_to(lb, (T, D))
            return None
        return pv_finish(h, o2, lt, lb)

    def pv_finish(h, o2, lt, lb):
        ot = osc[h, pl.ds(0, T, stride=2), :] * _recip(lt)
        ob = (osc[h, pl.ds(1, T, stride=2), :] + o2) * _recip(lb)
        return jnp.concatenate([ot, ob], axis=0).astype(bf16)

    def combine(i, a):
        rows = slice(i * TQ, (i + 1) * TQ)
        g = gbuf[rows, :]
        for jj in range(NJ):
            b = bbuf[jj, rows, :]
            obuf[rows, jj * T:(jj + 1) * T] = (b + g * (a[:, jj * T:(jj + 1) * T] - b)).astype(bf16)

    def oproj(i, ctx2, wo, s, final=False):
        rows = slice(i * TQ, (i + 1) * TQ)
        if final:
            combine(i, _nn(ctx2, wo) + acc[rows, :])
        else:
            acc[rows, :] = _nn(ctx2, wo) + jnp.where(s > 0, acc[rows, :], 0.0)

    def load_wo(s):
        return wo_s[pl.ds(2 * s, 2)].reshape(2 * D, M)

    def b_piece(s, a, prev):
        j = s // 2
        jl = pl.ds(_aligned(j * T, T), T)
        rows = slice(a * T, (a + 1) * T)
        taps = par_s[pl.ds(_aligned(j * 8, 8), 8), :]
        kf = bk_s[rows, jl].astype(f32)
        ks = kf * taps[0:1, :]
        tail = prev[1] if prev is not None else jnp.zeros((8, T), f32)
        ext = jnp.concatenate([tail, kf], axis=0)
        for t in range(1, KS):
            ks = ks + pltpu.roll(ext, t, 0)[8:, :] * taps[t:t + 1, :]
        u = ks * bv_s[rows, jl].astype(f32)
        ut[rows, :] = u * taps[KS:KS + 1, :]
        fm = f_s[s % 2]
        uh = _nn(fm, u.astype(bf16))
        ur, ui = uh[0:hf], uh[hf:T]
        bst[0, a] = ur
        bst[1, a] = ui
        bst[2, a] = ur + ui
        hh = _nt(fm, sk_s[pl.ds(_aligned(j * T, T), T), rows])
        hr, hi = hh[0:hf], hh[hf:T]
        if prev is not None:
            prev_h = prev[0]
            pr, pi = prev_h[0:hf], prev_h[hf:T]
            q = hf // 2
            hr = jnp.concatenate([hr[:q] - pi[:q], hr[q:] + pi[q:]], axis=0)
            hi = jnp.concatenate([hi[:q] + pr[:q], hi[q:] - pr[q:]], axis=0)
        bst[3, a] = hr
        bst[4, a] = hi - hr
        bst[5, a] = hr + hi
        return hh, kf[T - 8:, :]

    def b_front(s):
        ph = None
        for a in range(NC):
            ph = b_piece(s, a, ph)

    def b_mac(s, c, last=False):
        k1 = k2 = k3 = None
        for a in range(c + 1):
            jj = c - a
            t1 = bst[3, jj] * bst[2, a]
            t2 = bst[0, a] * bst[4, jj]
            t3 = bst[1, a] * bst[5, jj]
            k1 = t1 if k1 is None else k1 + t1
            k2 = t2 if k2 is None else k2 + t2
            k3 = t3 if k3 is None else k3 + t3
        z = jnp.concatenate([k1 - k3, k1 + k2], axis=0).astype(bf16)
        rows = slice(c * T, (c + 1) * T)
        y = _nn(gi_s[s % 2], z)
        if last:
            y = y + ybuf[rows, :]
        else:
            y = y + jnp.where(s % 2 == 1, ybuf[rows, :], 0.0)
            ybuf[rows, :] = y
        j = s // 2
        jl = pl.ds(_aligned(j * T, T), T)
        bbuf[j, rows, :] = x_s[rows, jl].astype(f32) * (y + ut[rows, :])

    def front_first():
        cp_c(0).start()
        for kind in (1, 2):
            zero_group0(kind)
            cp_pair0(kind).start()
        for i in range(1, NCC):
            cp_c(i).start()
        for i in range(5):
            cp_small(i).start()
        cp_x(NB - 1).start()
        for kind in range(3):
            cp_b(kind, 0).start()
        zero_group0(0)
        cp_pair0(0).start()
        for i in range(NB - 2, 1, -1):
            cp_x(i).start()
        cp_wo(0).start()
        cp_x(1).start()
        cp_x(0).start()

        cp_pair0(1).wait()
        convert_loop(1)
        cp_pair0(2).wait()
        convert_loop(2)
        cp_w(1, 0).start()
        cp_w(2, 0).start()
        rc = S // NCC

        def kv_chunk(i, carry):
            r = pl.ds(pl.multiple_of(i * rc, rc), rc)
            pltpu.make_async_copy(c_hbm.at[r, :], c_s.at[r, :], sems.at[SEM_C + i]).wait()
            cc = c_s[r, :]
            rp = pl.ds(pl.multiple_of(i * (rc // 2), rc // 2), rc // 2)
            c32[rp, :] = _pack(cc)
            kv32[0, rp, :] = _pack(_nn(cc, load_w(1, 0)).astype(bf16))
            kv32[1, rp, :] = _pack(_nn(cc, load_w(2, 0)).astype(bf16))
            return carry

        lax.fori_loop(0, NCC, kv_chunk, 0)
        cp_pair0(0).wait()
        convert_loop(0)
        cp_w(0, 0).start()
        cp_wo(1).start()
        for kind in range(3):
            cp_w(kind, 1).start()
        for kind in range(3):
            cp_b(kind, 1).start()
        cp_wo(2).start()
        for g in range(2, NG):
            for kind in range(3):
                cp_w(kind, g).start()
        for i in range(5):
            cp_small(i).wait()
        for kind in range(3):
            cp_b(kind, 0).wait()
        shf = sh_s[...].astype(f32)
        sdf = sd_s[...].astype(f32).reshape(1, M)
        for jj in range(NJ):
            par_s[jj * 8:jj * 8 + KS, :] = shf[:, jj * T:(jj + 1) * T]
            par_s[jj * 8 + KS:jj * 8 + KS + 1, :] = sdf[:, jj * T:(jj + 1) * T]
            par_s[jj * 8 + KS + 1:jj * 8 + 8, :] = jnp.zeros((8 - KS - 1, T), f32)
        x_ready(NB - 1)
        qa32[...] = _pack(qproj(NB - 1, load_w(0, 0)))
        b_front(0)
        x_ready_loop(NB - 2, NB - 3)
        cp_wo(0).wait()

    def seg_a(s):
        wq = load_w(0, s)
        wo = load_wo(s)
        qn = _unpack(qa32[...])
        prev = None
        for i in range(NB - 1, SPLIT - 1, -1):
            w = (i + 1) * TQ
            q2 = qn
            sc = [None, None]
            ctx = [None, None]
            for op in ORDER_A[i].split("."):
                if op == "SA":
                    sc[0] = scores(q2[:, 0:D], 0, w)
                elif op == "SB":
                    sc[1] = scores(q2[:, D:2 * D], 1, w)
                elif op[0] == "M":
                    b_mac(s, int(op[1:]))
                elif op == "Q":
                    qn = qproj(i - 1, wq)
                elif op == "PA":
                    ctx[0] = pv(sc[0], 0, w)
                elif op == "PB":
                    ctx[1] = pv(sc[1], 1, w, defer=(i == SPLIT))
                    if ctx[1] is None:
                        ctx[1] = ctx[0]
                elif op == "O":
                    if prev is not None:
                        oproj(i + 1, prev, wo, s)
            prev = jnp.concatenate(ctx, axis=1)
        qb32[...] = _pack(qn)
        cx32[...] = _pack(prev)

    def seg_b(s, last):
        if not last:
            sn = s + 1
            gsrc = jnp.minimum(s // P + 1, NG - 1)
            gdst = s // P + 1
            q4 = s % P
            for kind in range(3):
                n = w_rows[kind] // P
                convert(kind, gsrc, gdst, _aligned(q4 * n, n), n)
            wuk = load_w(1, sn)
            wuv = load_w(2, sn)
        wq = load_w(0, s)
        wo = load_wo(s)
        st = {"q": _unpack(qb32[...]), "prev": _unpack(cx32[...]), "h": None, "a": 0}
        st["prev"] = jnp.concatenate([st["prev"][:, 0:D], pv_finish(1, dsc[0], dsc[1], dsc[2])], axis=1)

        def job(name):
            kind, i = name[0], int(name[-1])
            if name[0] == "M":
                b_mac(s, i, last)
            elif name[:2] in ("SA", "SB"):
                h = 0 if name[1] == "A" else 1
                st["sc", h] = scores(st["q", i][:, h * D:(h + 1) * D], h, (i + 1) * TQ)
            elif kind == "Q":
                st["q", i] = qproj(i, wq)
            elif name[:2] in ("PA", "PB"):
                h = 0 if name[1] == "A" else 1
                st["ctx", i, h] = pv(st["sc", h], h, (i + 1) * TQ)
            elif kind == "O":
                ctx = st["prev"] if i == SPLIT else jnp.concatenate([st["ctx", i, 0], st["ctx", i, 1]], axis=1)
                oproj(i, ctx, wo, s, last)
            elif kind == "K":
                if not last:
                    kvproj(i, wuk, wuv)
            elif kind == "N":
                if not last:
                    qa32[...] = _pack(qproj(NB - 1, load_w(0, sn)))
            elif kind == "C":
                if last:
                    combine(i, acc[i * TQ:(i + 1) * TQ, :])
            elif kind == "D":
                if last:
                    cp_out(i).start()
            elif kind == "F":
                if not last:
                    for _ in range(i):
                        if st["a"] < NC:
                            st["h"] = b_piece(sn, st["a"], st["h"])
                            st["a"] += 1

        st["q", SPLIT - 1] = st["q"]
        jobs = (ORDER_LAST if last else ORDER_B).split(".")
        for name in jobs:
            job(name)
        if not last:
            assert st["a"] == NC, st["a"]
        else:
            for k in range(len(OUT_CHUNKS)):
                cp_out(k).wait()


    front_first()

    def step(s, carry):
        seg_a(s)

        @pl.when(jnp.logical_and(s <= (NG - 2) * P, jnp.logical_or(s <= 1, s % P == 0)))
        def _():
            @pl.when(s == 0)
            def _():
                x_ready_loop(1, 2)
                for kind in range(3):
                    cp_w(kind, 0).wait()
                    convert_loop(kind)
                cp_wo(1).wait()
                for kind in range(3):
                    cp_w(kind, 1).wait()

            @pl.when(s == 1)
            def _():
                cp_wo(2).wait()
                for kind in range(3):
                    cp_b(kind, 1).wait()

            for g in range(2, NG):
                @pl.when(s == (g - 1) * P)
                def _():
                    for kind in range(3):
                        cp_w(kind, g).wait()

        @pl.when(s < NS - 1)
        def _():
            seg_b(s, False)

        @pl.when(s == NS - 1)
        def _():
            seg_b(s, True)

        return carry

    lax.fori_loop(0, NS, step, 0)


@jax.jit
def pallas_gated_mix__compressed_kv_cla__ssm_conv_h3__prompt_kernel(
    A_x: jax.Array,
    A_c_kv: jax.Array,
    A_w_q: jax.Array,
    A_w_uk: jax.Array,
    A_w_uv: jax.Array,
    A_w_o: jax.Array,
    B_q: jax.Array,
    B_k: jax.Array,
    B_v: jax.Array,
    B_shift_k: jax.Array,
    B_ssm_k: jax.Array,
    B_ssm_D: jax.Array,
    gate_w: jax.Array,
):
    del B_q
    x = A_x.reshape(S, M)
    c = A_c_kv.reshape(S, C)
    bk = B_k.reshape(S, M)
    bv = B_v.reshape(S, M)
    sh = B_shift_k.T
    fwd, inv = _dft_tables()
    fwd = jnp.asarray(fwd, dtype=bf16)
    inv = jnp.asarray(inv, dtype=bf16)

    any_spec = pl.BlockSpec(memory_space=pl.ANY)
    out = pl.pallas_call(
        _kernel,
        in_specs=[any_spec] * 14,
        out_specs=any_spec,
        out_shape=jax.ShapeDtypeStruct((S, M), bf16),
        scratch_shapes=[
            pltpu.VMEM((S, M), bf16),
            pltpu.VMEM((S, C), bf16),
            pltpu.VMEM((NG, M, G, D), bf16),
            pltpu.VMEM((NG, C, G, D), bf16),
            pltpu.VMEM((NG, C, G, D), bf16),
            pltpu.VMEM((NG + 1, M * P, D), u32),
            pltpu.VMEM((NG + 1, C * P, D), u32),
            pltpu.VMEM((NG + 1, C * P, D), u32),
            pltpu.VMEM((H, D, M), bf16),
            pltpu.VMEM((S, M), bf16),
            pltpu.VMEM((S, M), bf16),
            pltpu.VMEM((M, S), bf16),
            pltpu.VMEM((KS, M), bf16),
            pltpu.VMEM((M,), bf16),
            pltpu.VMEM((M,), bf16),
            pltpu.VMEM((2, T, T), bf16),
            pltpu.VMEM((2, T, T), bf16),
            pltpu.VMEM((NJ * 8, T), f32),
            pltpu.VMEM((2, S // 2, 2 * D), u32),
            pltpu.VMEM((TQ // 2, 2 * D), u32),
            pltpu.VMEM((TQ // 2, 2 * D), u32),
            pltpu.VMEM((TQ // 2, 2 * D), u32),
            pltpu.VMEM((6, NC, T // 2, T), f32),
            pltpu.VMEM((S, T), f32),
            pltpu.VMEM((2, TQ, D), f32),
            pltpu.VMEM((S // 2, M), u32),
            pltpu.VMEM((S // 2, C), u32),
            pltpu.VMEM((3, T, D), f32),
            pltpu.VMEM((S, M), f32),
            pltpu.VMEM((S, T), f32),
            pltpu.VMEM((NJ, S, T), f32),
            pltpu.VMEM((S, T), f32),
            pltpu.VMEM((S, M), bf16),
            pltpu.SemaphoreType.DMA((NSEM,)),
        ],
        compiler_params=pltpu.CompilerParams(
            vmem_limit_bytes=120 * 1024 * 1024,
        ),
        name="gated_mix",
    )(x, c, A_w_q, A_w_uk, A_w_uv, A_w_o, bk, bv, B_ssm_k, sh, B_ssm_D, gate_w, fwd, inv)
    return out.reshape(1, S, M)
```
